```python
import jax
import jax.numpy as jnp

def _softmax(x, axis=-1):
    return jax.nn.softmax(x, axis=axis)

def _gelu(x):
    return jax.nn.gelu(x, approximate=True)

def _silu(x):
    return jax.nn.silu(x)

def _sigmoid(x):
    return jax.nn.sigmoid(x)

def _layernorm(x, axis=-1, eps=1e-05):
    m = jnp.mean(x, axis=axis, keepdims=True)
    v = jnp.var(x, axis=axis, keepdims=True)
    return (x - m) / jnp.sqrt(v + eps)

def _scatter_add(tgt, idx, src, axis=0):
    return tgt.at[idx].add(src)

def _segment_sum(src, seg, n):
    return jax.ops.segment_sum(src, seg, n)

class _Rng:

    def __init__(self, key):
        self._k = key

    def _next(self):
        self._k, sub = jax.random.split(self._k)
        return sub

    def normal(self, shape):
        return jax.random.normal(self._next(), shape, dtype=jnp.bfloat16)

    def randint(self, lo, hi, shape):
        return jax.random.randint(self._next(), shape, lo, hi, dtype=jnp.int32)

    def uniform(self, shape, lo=0.0, hi=1.0):
        return jax.random.uniform(self._next(), shape, jnp.bfloat16, lo, hi)

    def permutation(self, n):
        return jax.random.permutation(self._next(), n)
kernel_name = 'standalone__window_attn_davit__vision'

def setup_inputs():
    _rng = _Rng(jax.random.key(int.from_bytes(__import__("os").urandom(4), "little")))
    _w = lambda a: (lambda t: t.astype(jnp.bfloat16) if jnp.issubdtype(t.dtype, jnp.floating) else t)(jnp.asarray(a))
    HW = 512
    C0 = 192
    ws = 7
    nh = 4
    H = W = max(HW // ws * ws, ws)
    C = max(C0 // nh * nh, nh)
    k = 3
    return {'x': _w((lambda *s: _rng.normal(s) * 0.05)(1, H, W, C)), 'dw_pe': _w((lambda *s: _rng.normal(s) * 0.05)(k, k, C) * 0.1), 'w_qkv': _w((lambda *s: _rng.normal(s) * 0.05)(C, 3 * C) * C ** (-0.5)), 'w_o': _w((lambda *s: _rng.normal(s) * 0.05)(C, C) * C ** (-0.5))}

def reference(x, dw_pe, w_qkv, w_o):
    B, H, W, C = x.shape
    ws = 7
    nh = 4
    dh = C // nh
    kk = dw_pe.shape[0]
    pad = kk // 2
    xp = jnp.pad(x, ((0, 0), (pad, pad), (pad, pad), (0, 0)))
    pe = jnp.zeros_like(x)
    for i in range(kk):
        for j in range(kk):
            pe = pe + xp[:, i:i + H, j:j + W, :] * dw_pe[i, j][None, None, None, :]
    x0 = x + pe
    h = _layernorm(x0, axis=-1)
    hw = h.reshape(B, H // ws, ws, W // ws, ws, C)
    hw = (lambda x, *d: x.transpose(*d))(hw, 0, 1, 3, 2, 4, 5)
    hw = hw.reshape(-1, ws * ws, C)
    qkv = (hw @ w_qkv).reshape(-1, ws * ws, 3, nh, dh)
    q = qkv[:, :, 0].copy()
    k = qkv[:, :, 1].copy()
    v = qkv[:, :, 2].copy()
    scale = dh ** (-0.5)
    attn = jnp.einsum('wnhd,wmhd->whnm', q, k) * scale
    attn = _softmax(attn, axis=-1)
    out = jnp.einsum('whnm,wmhd->wnhd', attn, v)
    out = out.reshape(-1, ws * ws, C) @ w_o
    out = out.reshape(B, H // ws, W // ws, ws, ws, C)
    out = (lambda x, *d: x.transpose(*d))(out, 0, 1, 3, 2, 4, 5)
    out = out.reshape(B, H, W, C)
    return x0 + out
```

```python
import numpy as np
import jax
import jax.numpy as jnp
from jax import lax
import jax.experimental.pallas as pl
import jax.experimental.pallas.tpu as pltpu

WS = 7
NH = 4
C = 192
DH = C // NH
H = W = 511
WP = 512
NSTRIP = H // WS
NWIN = W // WS
NG = 5
GRP_TILES = (8, 8, 8, 8, 5)
LOG2E = 1.4426950408889634
EPS = 1e-5
U32 = jnp.uint32
F32 = jnp.float32
BF16 = jnp.bfloat16


def _fwd_pattern(g, r, par):
    lane = np.arange(128)
    bp, s, c = lane // 64, (lane // 8) % 8, lane % 8
    b = bp ^ par
    t = (s - r) % 8
    jj = 2 * t + b
    return ((112 * g + 7 * jj + np.minimum(c, 6)) % 128).astype(np.int32)


def _inv_pattern(g, r, par):
    idx = np.zeros(128, np.int32)
    for jj in range(16):
        t, b = jj // 2, jj % 2
        for c in range(7):
            p = (112 * g + 7 * jj + c) % 128
            idx[p] = 64 * (b ^ par) + 8 * ((t + r) % 8) + c
    return idx


def _pattern_table():
    rows = []
    for g in range(NG):
        for r in range(WS):
            for par in range(2):
                rows.append(_fwd_pattern(g, r, par))
    for g in range(NG):
        for r in range(WS):
            for par in range(2):
                rows.append(_inv_pattern(g, r, par))
    tab = np.stack(rows)
    return np.broadcast_to(tab[:, None, :], (tab.shape[0], 8, 128)).copy()


def _pidx(inv, g, r, par):
    return ((inv * NG + g) * WS + r) * 2 + par


def _barrel(ins, masks, nout):
    m1, m2, m4 = masks
    u = [ins[(-m) % 8] for m in range(8)]
    v1 = [jnp.where(m1, u[(t - 1) % 8], u[t]) for t in range(8)]
    v2 = [jnp.where(m2, v1[(t - 2) % 8], v1[t]) for t in range(8)]
    return [jnp.where(m4, v2[(t - 4) % 8], v2[t]) for t in range(nout)]


def _kernel(xm_ref, xt_ref, xb_ref, dw_ref, wt_ref, wo_ref, pat_ref, o_ref,
            wtab, wts, x0s, hs, gq, gv, kn, dq, dv, do, res):
    i = pl.program_id(0)

    @pl.when(i == 0)
    def _init():
        for k in range(9):
            w = dw_ref[k].astype(F32)
            if k == 4:
                w = w + 1.0
            wtab[k] = w
        wts[0:C, :] = (wt_ref[0:C, :].astype(F32) * (DH ** -0.5 * LOG2E)).astype(BF16)
        wts[C:3 * C, :] = wt_ref[C:3 * C, :]

    lane8 = lax.broadcasted_iota(jnp.int32, (8, 128), 1)
    lane512 = lax.broadcasted_iota(jnp.int32, (8, WP), 1)

    for rho in range(9):
        for ch in range(12):
            rs = pl.ds(16 * ch, 16)
            if rho == 0:
                xp = pltpu.bitcast(xt_ref[0, rs, :], U32)
                xp = jnp.where((lane512 < W) & (i > 0), xp, jnp.zeros_like(xp))
            elif rho == 8:
                xp = pltpu.bitcast(xb_ref[0, rs, :], U32)
                xp = jnp.where((lane512 < W) & (i < NSTRIP - 1), xp, jnp.zeros_like(xp))
            else:
                xp = pltpu.bitcast(xm_ref[rho - 1, rs, :], U32)
                last = jnp.where(lane8 < W - 384, xp[:, 384:], jnp.zeros_like(xp[:, 384:]))
                xp = jnp.concatenate([xp[:, :384], last], axis=1)
            xl = pltpu.roll(xp, 1, 1)
            xl = jnp.where(lane512 > 0, xl, jnp.zeros_like(xl))
            xr = pltpu.roll(xp, WP - 1, 1)
            xs = [pltpu.bitcast(v, BF16).astype(F32) for v in (xl, xp, xr)]
            for ki in range(3):
                r = rho - ki
                if r < 0 or r >= WS:
                    continue
                t = None
                for kj in range(3):
                    w = wtab[3 * ki + kj, rs, :]
                    w = jnp.concatenate([w] * 4, axis=1)
                    term = xs[kj] * w
                    t = term if t is None else t + term
                if ki == 0:
                    x0s[r, rs, :] = t
                else:
                    x0s[r, rs, :] = x0s[r, rs, :] + t

    for r in range(WS):
        for s in range(4):
            ls = pl.ds(128 * s, 128)
            x0 = x0s[r, :, ls]
            mean = jnp.sum(x0, axis=0, keepdims=True) * (1.0 / C)
            xc = x0 - mean
            var = jnp.sum(xc * xc, axis=0, keepdims=True) * (1.0 / C)
            hs[r, :, ls] = (xc * lax.rsqrt(var + EPS)).astype(BF16)

    offs = [(112 * g) // 128 for g in range(NG)], [(112 * g) % 128 for g in range(NG)]
    lane96 = lax.broadcasted_iota(jnp.int32, (24, 128), 1)
    for r in range(WS):
        h = hs[r]
        for part in range(6):
            y = jnp.dot(wts[pl.ds(96 * part, 96), :], h, preferred_element_type=F32)
            kind, pair = part // 2, part % 2
            if kind == 1:
                for s in range(4):
                    blk = jnp.concatenate(
                        [y[:, 128 * s:128 * (s + 1)], jnp.zeros((32, 128), F32)], axis=0)
                    kn[pair, r, pl.ds(128 * s, 128), :] = blk.T
            else:
                yp = pltpu.bitcast(y.astype(BF16), U32)
                dst = gq if kind == 0 else gv
                for hh in range(2):
                    par = hh if kind == 0 else 0
                    yh = yp[24 * hh:24 * (hh + 1)]
                    for g in range(NG):
                        a, off = offs[0][g], offs[1][g]
                        src = yh[:, 128 * a:128 * (a + 1)]
                        if g not in (0, NG - 1):
                            src = jnp.where(lane96 >= off, src, yh[:, 128 * (a + 1):128 * (a + 2)])
                        idx = pat_ref[_pidx(0, g, r, par)]
                        idx = jnp.concatenate([idx] * 3, axis=0)
                        row0 = 48 * pair + 24 * hh
                        dst[r, g, pl.ds(row0, 24), :] = jnp.take_along_axis(src, idx, axis=1)

    lane24 = lane96
    masks = (((lane24 >> 3) & 1) == 1, ((lane24 >> 4) & 1) == 1, ((lane24 >> 5) & 1) == 1)
    zero24 = jnp.zeros((24, 128), U32)
    for src, dst in ((gq, dq), (gv, dv)):
        for g in range(NG):
            for hd in range(NH):
                rs = pl.ds(24 * hd, 24)
                ins = [src[r, g, rs, :] for r in range(WS)] + [zero24]
                outs = _barrel(ins, masks, GRP_TILES[g])
                for t, v in enumerate(outs):
                    dst[g, t, rs, :] = v

    lo96 = lax.broadcasted_iota(jnp.int32, (48, 128), 1) < 64
    lo64 = lax.broadcasted_iota(jnp.int32, (32, 128), 1) < 64
    lo1 = lax.broadcasted_iota(jnp.int32, (1, 128), 1) < 64
    kvalid = (lax.broadcasted_iota(jnp.int32, (56, 128), 0) & 7) < 7
    zero48 = jnp.zeros((48, 128), U32)
    zero32 = jnp.zeros((32, 128), U32)
    zero8f = jnp.zeros((8, 128), F32)
    row48 = lax.broadcasted_iota(jnp.int32, (48, 128), 0) < 24
    for g in range(NG):
        for t in range(GRP_TILES[g]):
            padslot = (t + 7) % 8
            for pair in range(2):
                q = dq[g, t, pl.ds(48 * pair, 48), :]
                keep_a = lo96 == row48
                ra = jnp.where(keep_a, q, zero48)
                rb = jnp.where(keep_a, zero48, q)
                ps, ls_ = [], []
                for b, rq in ((0, ra), (1, rb)):
                    j = 16 * g + 2 * t + b
                    j = min(j, NWIN - 1)
                    pieces = []
                    for s in range(8):
                        r = (s - t) % 8
                        pieces.append(zero8f if r == 7 else kn[pair, r, pl.ds(7 * j, 8), :])
                    kk = jnp.concatenate(pieces, axis=0).astype(BF16)
                    rq = pltpu.bitcast(rq, BF16)
                    sc = jnp.dot(kk[:, :96], rq, preferred_element_type=F32)
                    sc = jnp.concatenate(
                        [sc[8 * s:8 * s + 8] for s in range(8) if s != padslot], axis=0)
                    sc = jnp.where(kvalid, sc, -jnp.inf)
                    m = jnp.max(sc, axis=0, keepdims=True)
                    p = jnp.exp2(sc - m)
                    ls_.append(jnp.sum(p, axis=0, keepdims=True))
                    blocks = []
                    k = 0
                    for s in range(8):
                        if s == padslot:
                            blocks.append(zero8f)
                        else:
                            blocks.append(p[8 * k:8 * k + 8])
                            k += 1
                    pf = jnp.concatenate(blocks, axis=0).astype(BF16)
                    ps.append(pltpu.bitcast(pf, U32))
                for hh in range(2):
                    if hh == 0:
                        pa = jnp.where(lo64, ps[0], zero32)
                        pb = jnp.where(lo64, zero32, ps[1])
                        l = jnp.where(lo1, ls_[0], ls_[1])
                    else:
                        pa = jnp.where(lo64, zero32, ps[0])
                        pb = jnp.where(lo64, ps[1], zero32)
                        l = jnp.where(lo1, ls_[1], ls_[0])
                    pfull = pltpu.bitcast(jnp.concatenate([pa, pb], axis=0), BF16)
                    v = pltpu.bitcast(dv[g, t, pl.ds(48 * pair + 24 * hh, 24), :], BF16)
                    o = jnp.dot(v, pfull, preferred_element_type=F32)
                    o = o * pl.reciprocal(l, approx=False)
                    do[g, t, pl.ds(48 * pair + 24 * hh, 24), :] = pltpu.bitcast(o.astype(BF16), U32)

    for g in range(NG):
        for hd in range(NH):
            rs = pl.ds(24 * hd, 24)
            ins = [do[g, t, rs, :] if t < GRP_TILES[g] else zero24 for t in range(8)]
            outs = _barrel(ins, masks, WS)
            for r, v in enumerate(outs):
                idx = pat_ref[_pidx(1, g, r, hd % 2)]
                idx = jnp.concatenate([idx] * 3, axis=0)
                res[r, g, rs, :] = jnp.take_along_axis(v, idx, axis=1)

    lane96f = lax.broadcasted_iota(jnp.int32, (96, 128), 1)
    bounds = (112, 96, 80, 64)
    for r in range(WS):
        tiles = [jnp.where(lane96f < bounds[s], res[r, s], res[r, s + 1]) for s in range(4)]
        oimg = pltpu.bitcast(jnp.concatenate(tiles, axis=1), BF16)
        y = jnp.dot(wo_ref[...], oimg, preferred_element_type=F32)
        o_ref[r] = (y + x0s[r]).astype(o_ref.dtype)


@jax.jit
def pallas_standalone__window_attn_davit__vision_kernel(x, dw_pe, w_qkv, w_o):
    B, Hh, Ww, Cc = x.shape
    assert (B, Hh, Ww, Cc) == (1, H, W, C)
    xt = jnp.transpose(x, (0, 1, 3, 2)).reshape(H, C, W)
    dwb = jnp.broadcast_to(dw_pe.reshape(9, C, 1), (9, C, 128))
    wt = jnp.transpose(w_qkv)
    wo = jnp.transpose(w_o)
    pat = jnp.asarray(_pattern_table())

    last = H - 1
    out = pl.pallas_call(
        _kernel,
        grid=(NSTRIP,),
        in_specs=[
            pl.BlockSpec((WS, C, WP), lambda i: (i, 0, 0)),
            pl.BlockSpec((1, C, WP), lambda i: (jnp.maximum(WS * i - 1, 0), 0, 0)),
            pl.BlockSpec((1, C, WP), lambda i: (jnp.minimum(WS * i + WS, last), 0, 0)),
            pl.BlockSpec((9, C, 128), lambda i: (0, 0, 0)),
            pl.BlockSpec((3 * C, C), lambda i: (0, 0)),
            pl.BlockSpec((C, C), lambda i: (0, 0)),
            pl.BlockSpec(pat.shape, lambda i: (0, 0, 0)),
        ],
        out_specs=pl.BlockSpec((WS, C, WP), lambda i: (i, 0, 0)),
        out_shape=jax.ShapeDtypeStruct((H, C, W), x.dtype),
        scratch_shapes=[
            pltpu.VMEM((9, C, 128), F32),
            pltpu.VMEM((3 * C, C), BF16),
            pltpu.VMEM((WS, C, WP), F32),
            pltpu.VMEM((WS, C, WP), BF16),
            pltpu.VMEM((WS, NG, 96, 128), U32),
            pltpu.VMEM((WS, NG, 96, 128), U32),
            pltpu.VMEM((2, WS, WP, 128), F32),
            pltpu.VMEM((NG, 8, 96, 128), U32),
            pltpu.VMEM((NG, 8, 96, 128), U32),
            pltpu.VMEM((NG, 8, 96, 128), U32),
            pltpu.VMEM((WS, NG, 96, 128), U32),
        ],
        compiler_params=pltpu.CompilerParams(
            dimension_semantics=("arbitrary",),
            vmem_limit_bytes=100 * 1024 * 1024,
        ),
    )(xt, xt, xt, dwb, wt, wo, pat)
    return jnp.transpose(out.reshape(1, H, C, W), (0, 1, 3, 2))
```

```python
import numpy as np
import jax
import jax.numpy as jnp
from jax import lax
import jax.experimental.pallas as pl
import jax.experimental.pallas.tpu as pltpu

WS = 7
NH = 4
C = 192
DH = C // NH
H = W = 511
WP = 512
NSTRIP = H // WS
NWIN = W // WS
NG = 5
GRP_TILES = (8, 8, 8, 8, 5)
LOG2E = 1.4426950408889634
EPS = 1e-5
U32 = jnp.uint32
F32 = jnp.float32
BF16 = jnp.bfloat16
BLOCK_BARRIER = False


def _fwd_pattern(g, r, par):
    lane = np.arange(128)
    bp, s, c = lane // 64, (lane // 8) % 8, lane % 8
    b = bp ^ par
    t = (s - r) % 8
    jj = 2 * t + b
    return ((112 * g + 7 * jj + np.minimum(c, 6)) % 128).astype(np.int32)


def _inv_pattern(g, r, par):
    idx = np.zeros(128, np.int32)
    for jj in range(16):
        t, b = jj // 2, jj % 2
        for c in range(7):
            p = (112 * g + 7 * jj + c) % 128
            idx[p] = 64 * (b ^ par) + 8 * ((t + r) % 8) + c
    return idx


def _pattern_table():
    rows = []
    for g in range(NG):
        for r in range(WS):
            for par in range(2):
                rows.append(_fwd_pattern(g, r, par))
    for g in range(NG):
        for r in range(WS):
            for par in range(2):
                rows.append(_inv_pattern(g, r, par))
    tab = np.stack(rows)
    return np.broadcast_to(tab[:, None, :], (tab.shape[0], 8, 128)).copy()


def _pidx(inv, g, r, par):
    return ((inv * NG + g) * WS + r) * 2 + par


def _barrel(ins, masks, nout):
    m1, m2, m4 = masks
    u = [ins[(-m) % 8] for m in range(8)]
    v1 = [jnp.where(m1, u[(t - 1) % 8], u[t]) for t in range(8)]
    v2 = [jnp.where(m2, v1[(t - 2) % 8], v1[t]) for t in range(8)]
    return [jnp.where(m4, v2[(t - 4) % 8], v2[t]) for t in range(nout)]


def _kernel(xm_ref, xt_ref, xb_ref, dw_ref, wt_ref, wo_ref, pat_ref, o_ref,
            wtab, wts, wos, x0s, hs, gq, gv, kn, dq, dv, do, scs, res):
    i = pl.program_id(0)
    one = jnp.where(i >= 0, 1, 0)

    @pl.when(i == 0)
    def _init():
        for k in range(9):
            w = dw_ref[k].astype(F32)
            if k == 4:
                w = w + 1.0
            wtab[k] = jnp.concatenate([w] * 4, axis=1)
        src = lax.broadcasted_iota(jnp.int32, (C, C), 0)
        pos = lax.broadcasted_iota(jnp.int32, (C, C), 1)
        p_chan = (src == (pos >> 1) + 96 * (pos & 1)).astype(BF16)
        hd, within = pos // DH, pos % DH
        p_head = (src == hd * DH + (within >> 1) + 24 * (within & 1)).astype(BF16)
        wt = jnp.dot(wt_ref[...], p_chan, preferred_element_type=F32).astype(BF16)
        r_pos = lax.broadcasted_iota(jnp.int32, (C, C), 0)
        r_src = lax.broadcasted_iota(jnp.int32, (C, C), 1)
        r_in = r_pos % DH
        p_rows = (r_src == (r_pos // DH) * DH + 2 * (r_in % 24) + r_in // 24).astype(BF16)
        wq = jnp.dot(p_rows, wt[0:C], preferred_element_type=F32)
        wts[0:C, :] = (wq * (DH ** -0.5 * LOG2E)).astype(BF16)
        wts[C:2 * C, :] = wt[C:2 * C]
        wts[2 * C:3 * C, :] = jnp.dot(p_rows, wt[2 * C:3 * C],
                                      preferred_element_type=F32).astype(BF16)
        wos[...] = jnp.dot(wo_ref[...], p_head, preferred_element_type=F32).astype(BF16)

    lane8 = lax.broadcasted_iota(jnp.int32, (8, 128), 1)
    lane512 = lax.broadcasted_iota(jnp.int32, (8, WP), 1)

    for rho in range(9):
        for ch in range(12):
            rs = pl.ds(16 * ch, 16)
            if rho == 0:
                xp = pltpu.bitcast(xt_ref[0, rs, :], U32)
                xp = jnp.where((lane512 < W) & (i > 0), xp, jnp.zeros_like(xp))
            elif rho == 8:
                xp = pltpu.bitcast(xb_ref[0, rs, :], U32)
                xp = jnp.where((lane512 < W) & (i < NSTRIP - 1), xp, jnp.zeros_like(xp))
            else:
                xp = pltpu.bitcast(xm_ref[rho - 1, rs, :], U32)
                last = jnp.where(lane8 < W - 384, xp[:, 384:], jnp.zeros_like(xp[:, 384:]))
                xp = jnp.concatenate([xp[:, :384], last], axis=1)
            xl = pltpu.roll(xp, 1, 1)
            xl = jnp.where(lane512 > 0, xl, jnp.zeros_like(xl))
            xr = pltpu.roll(xp, WP - 1, 1)
            xs = [pltpu.bitcast(v, BF16).astype(F32) for v in (xl, xp, xr)]
            for ki in range(3):
                r = rho - ki
                if r < 0 or r >= WS:
                    continue
                t = None
                for kj in range(3):
                    w = wtab[3 * ki + kj, rs, :]
                    term = xs[kj] * w
                    t = term if t is None else t + term
                if ki == 0:
                    x0s[r, rs, :] = t
                else:
                    x0s[r, rs, :] = x0s[r, rs, :] + t

    for r in range(WS):
        for s in range(4):
            ls = pl.ds(128 * s, 128)
            x0 = x0s[r, :, ls]
            mean = jnp.sum(x0, axis=0, keepdims=True) * (1.0 / C)
            xc = x0 - mean
            var = jnp.sum(xc * xc, axis=0, keepdims=True) * (1.0 / C)
            hn = xc * lax.rsqrt(var + EPS)
            hs[r, :, ls] = pltpu.pack_elementwise([hn[:96], hn[96:]], packed_dtype=BF16)

    offs = [(112 * g) // 128 for g in range(NG)], [(112 * g) % 128 for g in range(NG)]
    lane1 = lax.broadcasted_iota(jnp.int32, (1, 128), 1)
    for r in range(WS):
        h = pltpu.bitcast(hs[r], BF16)
        for part in range(6):
            y = jnp.dot(wts[pl.ds(96 * part, 96), :], h, preferred_element_type=F32)
            kind, pair = part // 2, part % 2
            if kind == 1:
                for s in range(4):
                    blk = jnp.concatenate(
                        [y[:, 128 * s:128 * (s + 1)], jnp.zeros((32, 128), F32)], axis=0)
                    kn[pair, r, pl.ds(128 * s, 128), :] = blk.T
            else:
                dst = gq if kind == 0 else gv
                for hh in range(2):
                    par = hh if kind == 0 else 0
                    yh = pltpu.pack_elementwise(
                        [y[48 * hh:48 * hh + 24], y[48 * hh + 24:48 * hh + 48]],
                        packed_dtype=BF16)
                    for g in range(NG):
                        a, off = offs[0][g], offs[1][g]
                        src = yh[:, 128 * a:128 * (a + 1)]
                        if g not in (0, NG - 1):
                            src = jnp.where(lane1 >= off, src, yh[:, 128 * (a + 1):128 * (a + 2)])
                        idx = pat_ref[_pidx(0, g, r, par)]
                        idx = jnp.concatenate([idx] * 3, axis=0)
                        row0 = 48 * pair + 24 * hh
                        dst[r, g, pl.ds(row0, 24), :] = jnp.take_along_axis(src, idx, axis=1)

    masks = (((lane1 >> 3) & 1) == 1, ((lane1 >> 4) & 1) == 1, ((lane1 >> 5) & 1) == 1)
    zero24 = jnp.zeros((24, 128), U32)
    for src, dst in ((gq, dq), (gv, dv)):
        for g in range(NG):
            for hd in range(NH):
                rs = pl.ds(24 * hd, 24)
                ins = [src[r, g, rs, :] for r in range(WS)] + [zero24]
                outs = _barrel(ins, masks, GRP_TILES[g])
                for t, v in enumerate(outs):
                    dst[g, t, rs, :] = v

    lo = lane1 < 64
    kvalid = (lax.broadcasted_iota(jnp.int32, (56, 128), 0) & 7) < 7
    zero16 = jnp.zeros((16, 128), U32)
    zero8f = jnp.zeros((8, 128), F32)

    def scores(g):
        for t in range(GRP_TILES[g]):
            padslot = (t + 7) % 8
            for pair in range(2):
                qe = dq[g, t, pl.ds(48 * pair, 24), :]
                qo = dq[g, t, pl.ds(48 * pair + 24, 24), :]
                ra = jnp.concatenate(
                    [jnp.where(lo, qe, zero24), jnp.where(lo, zero24, qo), zero16], axis=0)
                rb = jnp.concatenate(
                    [jnp.where(lo, zero24, qe), jnp.where(lo, qo, zero24), zero16], axis=0)
                for b, rq in ((0, ra), (1, rb)):
                    j = min(16 * g + 2 * t + b, NWIN - 1)
                    pieces = []
                    for s in range(8):
                        r = (s - t) % 8
                        pieces.append(zero8f if r == 7 else kn[pair, r, pl.ds(7 * j, 8), :])
                    kk = jnp.concatenate(pieces, axis=0).astype(BF16)
                    sc = jnp.dot(kk, pltpu.bitcast(rq, BF16), preferred_element_type=F32)
                    scs[g % 2, t, pair, b] = jnp.concatenate(
                        [sc[8 * s:8 * s + 8] for s in range(8) if s != padslot], axis=0)

    def softmax_pv(g):
        for t in range(GRP_TILES[g]):
            padslot = (t + 7) % 8
            for pair in range(2):
                ps, ls_ = [], []
                for b in range(2):
                    sc = jnp.where(kvalid, scs[g % 2, t, pair, b], -jnp.inf)
                    m = jnp.max(sc, axis=0, keepdims=True)
                    p = jnp.exp2(sc - m)
                    ls_.append(jnp.sum(p, axis=0, keepdims=True))
                    blocks, k = [], 0
                    for s in range(8):
                        if s == padslot:
                            blocks.append(zero8f)
                        else:
                            blocks.append(p[8 * k:8 * k + 8])
                            k += 1
                    ps.append(jnp.concatenate(blocks, axis=0))
                for hh in range(2):
                    if hh == 0:
                        pa = jnp.where(lo, ps[0], 0.0)
                        pb = jnp.where(lo, 0.0, ps[1])
                        l = jnp.where(lo, ls_[0], ls_[1])
                    else:
                        pa = jnp.where(lo, 0.0, ps[0])
                        pb = jnp.where(lo, ps[1], 0.0)
                        l = jnp.where(lo, ls_[1], ls_[0])
                    pfull = jnp.concatenate([pa, pb], axis=0).astype(BF16)
                    v = pltpu.bitcast(dv[g, t, pl.ds(48 * pair + 24 * hh, 24), :], BF16)
                    o = jnp.dot(v, pfull, preferred_element_type=F32)
                    rl = pltpu.reciprocal(l, approx=True)
                    rl = rl * (2.0 - l * rl)
                    o = o * rl
                    do[g, t, pl.ds(48 * pair + 24 * hh, 24), :] = pltpu.pack_elementwise(
                        [o[:24], o[24:]], packed_dtype=BF16)

    def block(fn):
        if BLOCK_BARRIER:
            lax.fori_loop(0, one, lambda _, c: (fn(), c)[1], 0)
        else:
            fn()

    block(lambda: scores(0))
    for g in range(NG):
        def step(g=g):
            if g + 1 < NG:
                scores(g + 1)
            softmax_pv(g)
        block(step)

    for g in range(NG):
        for hd in range(NH):
            rs = pl.ds(24 * hd, 24)
            ins = [do[g, t, rs, :] if t < GRP_TILES[g] else zero24 for t in range(8)]
            outs = _barrel(ins, masks, WS)
            for r, v in enumerate(outs):
                idx = pat_ref[_pidx(1, g, r, hd % 2)]
                idx = jnp.concatenate([idx] * 3, axis=0)
                res[r, g, rs, :] = jnp.take_along_axis(v, idx, axis=1)

    bounds = (112, 96, 80, 64)
    for r in range(WS):
        tiles = [jnp.where(lane1 < bounds[s], res[r, s], res[r, s + 1]) for s in range(4)]
        oimg = pltpu.bitcast(jnp.concatenate(tiles, axis=1), BF16)
        y = jnp.dot(wos[...], oimg, preferred_element_type=F32)
        o_ref[r] = (y + x0s[r]).astype(o_ref.dtype)


@jax.jit
def pallas_standalone__window_attn_davit__vision_kernel(x, dw_pe, w_qkv, w_o):
    B, Hh, Ww, Cc = x.shape
    assert (B, Hh, Ww, Cc) == (1, H, W, C)
    xt = jnp.transpose(x, (0, 1, 3, 2)).reshape(H, C, W)
    dwb = jnp.broadcast_to(dw_pe.reshape(9, C, 1), (9, C, 128))
    wt = jnp.transpose(w_qkv)
    wo = jnp.transpose(w_o)
    pat = jnp.asarray(_pattern_table())

    last = H - 1
    out = pl.pallas_call(
        _kernel,
        grid=(NSTRIP,),
        in_specs=[
            pl.BlockSpec((WS, C, WP), lambda i: (i, 0, 0)),
            pl.BlockSpec((1, C, WP), lambda i: (jnp.maximum(WS * i - 1, 0), 0, 0)),
            pl.BlockSpec((1, C, WP), lambda i: (jnp.minimum(WS * i + WS, last), 0, 0)),
            pl.BlockSpec((9, C, 128), lambda i: (0, 0, 0)),
            pl.BlockSpec((3 * C, C), lambda i: (0, 0)),
            pl.BlockSpec((C, C), lambda i: (0, 0)),
            pl.BlockSpec(pat.shape, lambda i: (0, 0, 0)),
        ],
        out_specs=pl.BlockSpec((WS, C, WP), lambda i: (i, 0, 0)),
        out_shape=jax.ShapeDtypeStruct((H, C, W), x.dtype),
        scratch_shapes=[
            pltpu.VMEM((9, C, WP), F32),
            pltpu.VMEM((3 * C, C), BF16),
            pltpu.VMEM((C, C), BF16),
            pltpu.VMEM((WS, C, WP), F32),
            pltpu.VMEM((WS, C // 2, WP), U32),
            pltpu.VMEM((WS, NG, 96, 128), U32),
            pltpu.VMEM((WS, NG, 96, 128), U32),
            pltpu.VMEM((2, WS, WP, 128), F32),
            pltpu.VMEM((NG, 8, 96, 128), U32),
            pltpu.VMEM((NG, 8, 96, 128), U32),
            pltpu.VMEM((NG, 8, 96, 128), U32),
            pltpu.VMEM((2, 8, 2, 2, 56, 128), F32),
            pltpu.VMEM((WS, NG, 96, 128), U32),
        ],
        compiler_params=pltpu.CompilerParams(
            dimension_semantics=("arbitrary",),
            vmem_limit_bytes=100 * 1024 * 1024,
        ),
    )(xt, xt, xt, dwb, wt, wo, pat)
    return jnp.transpose(out.reshape(1, H, C, W), (0, 1, 3, 2))
```

```python
import numpy as np
import jax
import jax.numpy as jnp
from jax import lax
import jax.experimental.pallas as pl
import jax.experimental.pallas.tpu as pltpu

WS = 7
NH = 4
C = 192
DH = C // NH
H = W = 511
WP = 512
NSTRIP = H // WS
NWIN = W // WS
NG = 5
GRP_TILES = (8, 8, 8, 8, 5)
LOG2E = 1.4426950408889634
EPS = 1e-5
U32 = jnp.uint32
F32 = jnp.float32
BF16 = jnp.bfloat16


def _fwd_pattern(g, r, par):
    lane = np.arange(128)
    bp, s, c = lane // 64, (lane // 8) % 8, lane % 8
    b = bp ^ par
    t = (s - r) % 8
    jj = 2 * t + b
    return ((112 * g + 7 * jj + np.minimum(c, 6)) % 128).astype(np.int32)


def _inv_pattern(g, r, par):
    idx = np.zeros(128, np.int32)
    for jj in range(16):
        t, b = jj // 2, jj % 2
        for c in range(7):
            p = (112 * g + 7 * jj + c) % 128
            idx[p] = 64 * (b ^ par) + 8 * ((t + r) % 8) + c
    return idx


def _pattern_table():
    rows = []
    for g in range(NG):
        for r in range(WS):
            for par in range(2):
                rows.append(_fwd_pattern(g, r, par))
    for g in range(NG):
        for r in range(WS):
            for par in range(2):
                rows.append(_inv_pattern(g, r, par))
    tab = np.stack(rows)
    return np.broadcast_to(tab[:, None, :], (tab.shape[0], 8, 128)).copy()


def _pidx(inv, g, r, par):
    return ((inv * NG + g) * WS + r) * 2 + par


def _hpos(hd):
    return 48 * (hd % 2) + 24 * (hd // 2)


def _barrel(ins, masks, nout):
    m1, m2, m4 = masks
    u = [ins[(-m) % 8] for m in range(8)]
    v1 = [jnp.where(m1, u[(t - 1) % 8], u[t]) for t in range(8)]
    v2 = [jnp.where(m2, v1[(t - 2) % 8], v1[t]) for t in range(8)]
    return [jnp.where(m4, v2[(t - 4) % 8], v2[t]) for t in range(nout)]


def _kernel(x0_ref, x1_ref, x2_ref, xa_ref, xb_ref, xc_ref, xd_ref, xe_ref, xf_ref, xg_ref,
            dw_ref, wt_ref, wo_ref, pat_ref, o_ref,
            wtab, wts, wos, x0s, xcs, x0n, hs, gq, gv, kn, dq, dv, do, scs, res, ob):
    i = pl.program_id(0)
    one = jnp.where(i >= 0, 1, 0)
    xrows = (xa_ref, xb_ref, xc_ref, xd_ref, xe_ref, xf_ref, xg_ref)

    lane1 = lax.broadcasted_iota(jnp.int32, (1, 128), 1)
    lane512 = lax.broadcasted_iota(jnp.int32, (1, WP), 1)

    def block(fn):
        lax.fori_loop(0, one, lambda _, c: (fn(), c)[1], 0)

    def conv_row(x_ref, valid, taps):
        for ch in range(12):
            rs = pl.ds(16 * ch, 16)
            xp = pltpu.bitcast(x_ref[0, rs, :], U32)
            if valid is None:
                last = jnp.where(lane1 < W - 384, xp[:, 384:], jnp.zeros_like(xp[:, 384:]))
                xp = jnp.concatenate([xp[:, :384], last], axis=1)
            else:
                xp = jnp.where((lane512 < W) & valid, xp, jnp.zeros_like(xp))
            xl = pltpu.roll(xp, 1, 1)
            first = jnp.where(lane1 > 0, xl[:, :128], jnp.zeros_like(xl[:, :128]))
            xl = jnp.concatenate([first, xl[:, 128:]], axis=1)
            xr = pltpu.roll(xp, WP - 1, 1)
            ws = [wtab[k, rs, :] for k in range(9)]
            for s_ in range(4):
                ls = pl.ds(128 * s_, 128)
                xs = [pltpu.bitcast(v[:, 128 * s_:128 * (s_ + 1)], BF16).astype(F32)
                      for v in (xl, xp, xr)]
                for ki, tap in enumerate(taps):
                    if tap is None:
                        continue
                    dst, src = tap
                    t = xs[0] * ws[3 * ki] + xs[1] * ws[3 * ki + 1] + xs[2] * ws[3 * ki + 2]
                    dst[rs, ls] = t if src is None else src[rs, ls] + t

    def layer_norm(x0_row, q):
        for s in range(4):
            ls = pl.ds(128 * s, 128)
            x0 = x0_row[:, ls]
            mean = jnp.sum(x0, axis=0, keepdims=True) * (1.0 / C)
            xc = x0 - mean
            var = jnp.sum(xc * xc, axis=0, keepdims=True) * (1.0 / C)
            hn = xc * lax.rsqrt(var + EPS)
            hs[q, :, ls] = pltpu.pack_elementwise([hn[:96], hn[96:]], packed_dtype=BF16)

    @pl.when(i == 0)
    def _init():
        for k in range(9):
            w = dw_ref[k].astype(F32)
            if k == 4:
                w = w + 1.0
            wtab[k] = w
        src = lax.broadcasted_iota(jnp.int32, (C, C), 0)
        pos = lax.broadcasted_iota(jnp.int32, (C, C), 1)
        p_chan = (src == (pos >> 1) + 96 * (pos & 1)).astype(BF16)
        hp, within = pos // DH, pos % DH
        hd = 2 * (hp % 2) + hp // 2
        p_head = (src == hd * DH + (within >> 1) + 24 * (within & 1)).astype(BF16)
        wt = jnp.dot(wt_ref[...], p_chan, preferred_element_type=F32).astype(BF16)
        r_in, r_hp = src % DH, src // DH
        r_hd = 2 * (r_hp % 2) + r_hp // 2
        p_rows = (pos == r_hd * DH + 2 * (r_in % 24) + r_in // 24).astype(BF16)
        wq = jnp.dot(p_rows, wt[0:C], preferred_element_type=F32)
        wts[0:C, :] = (wq * (DH ** -0.5 * LOG2E)).astype(BF16)
        wts[C:2 * C, :] = wt[C:2 * C]
        wts[2 * C:3 * C, :] = jnp.dot(p_rows, wt[2 * C:3 * C],
                                      preferred_element_type=F32).astype(BF16)
        wos[...] = jnp.dot(wo_ref[...], p_head, preferred_element_type=F32).astype(BF16)
        n0, n1, c0, c1 = x0n.at[0], x0n.at[1], xcs.at[0], xcs.at[1]
        conv_row(x0_ref, None, ((n1, None), (n0, None), None))
        conv_row(x1_ref, None, ((c0, None), (n1, n1), (n0, n0)))
        conv_row(x2_ref, None, ((c1, None), (c0, c0), (n1, n1)))
        layer_norm(n0, 0)

    offs = [((112 * g) // 128, (112 * g) % 128) for g in range(NG)]

    def gather_qv(yh, dst, r, rows, par):
        for g in range(NG):
            a, off = offs[g]
            src = yh[:, 128 * a:128 * (a + 1)]
            if g not in (0, NG - 1):
                src = jnp.where(lane1 >= off, src, yh[:, 128 * (a + 1):128 * (a + 2)])
            idx = jnp.concatenate([pat_ref[_pidx(0, g, r, par)]] * 6, axis=0)
            dst[r, g, rows, :] = jnp.take_along_axis(src, idx, axis=1)

    def qkv_row(r):
        h = pltpu.bitcast(hs[r], BF16)
        yk = jnp.dot(wts[C:2 * C, :], h, preferred_element_type=F32)
        kp = pltpu.pack_elementwise([yk[:96], yk[96:]], packed_dtype=BF16)
        for s in range(4):
            blk = jnp.concatenate(
                [kp[:, 128 * s:128 * (s + 1)], jnp.zeros((32, 128), U32)], axis=0)
            kn[r, pl.ds(128 * s, 128), :] = blk.T
        for part in (0, 1, 4, 5):
            y = jnp.dot(wts[pl.ds(96 * part, 96), :], h, preferred_element_type=F32)
            yh = jnp.concatenate([
                pltpu.pack_elementwise([y[48 * hh:48 * hh + 24], y[48 * hh + 24:48 * hh + 48]],
                                       packed_dtype=BF16) for hh in range(2)], axis=0)
            cls = part % 2
            gather_qv(yh, gq if part < 2 else gv, r, pl.ds(48 * cls, 48), cls if part < 2 else 0)

    def part(q):
        if 4 <= q <= 6:
            return x0s.at[q]
        return x0n.at[q - 7] if q in (7, 8) else xcs.at[(q - 2) % WS]

    def final(q):
        if 2 <= q <= 6:
            return x0s.at[q]
        return x0n.at[q % WS]

    for r in range(WS):
        def stage_a(r=r):
            valid = None if r < 4 else (WS * i + 3 + r < H)
            qkv_row(r)
            layer_norm(final(r + 1), (r + 1) % WS)
            if r < 2:
                x0s[r] = x0n[r]
            conv_row(xrows[r], valid, ((part(r + 4), None), (part(r + 3), part(r + 3)),
                                       (final(r + 2), part(r + 2))))
        stage_a()

    masks = (((lane1 >> 3) & 1) == 1, ((lane1 >> 4) & 1) == 1, ((lane1 >> 5) & 1) == 1)
    zero24 = jnp.zeros((24, 128), U32)
    zero16 = jnp.zeros((16, 128), U32)
    zero8f = jnp.zeros((8, 128), F32)
    lo = lane1 < 64
    kvalid = (lax.broadcasted_iota(jnp.int32, (56, 128), 0) & 7) < 7

    def regroup(src, dst, g):
        for hd in range(NH):
            rs = pl.ds(24 * hd, 24)
            ins = [src[r, g, rs, :] for r in range(WS)] + [zero24]
            for t, v in enumerate(_barrel(ins, masks, GRP_TILES[g])):
                dst[g, t, rs, :] = v

    def scores(g):
        for t in range(GRP_TILES[g]):
            padslot = (t + 7) % 8
            for pair in range(2):
                qe = dq[g, t, pl.ds(_hpos(2 * pair), 24), :]
                qo = dq[g, t, pl.ds(_hpos(2 * pair + 1), 24), :]
                ra = jnp.concatenate(
                    [jnp.where(lo, qe, zero24), jnp.where(lo, zero24, qo), zero16], axis=0)
                rb = jnp.concatenate(
                    [jnp.where(lo, zero24, qe), jnp.where(lo, qo, zero24), zero16], axis=0)
                for b, rq in ((0, ra), (1, rb)):
                    j = min(16 * g + 2 * t + b, NWIN - 1)
                    pieces = []
                    for s in range(8):
                        r = (s - t) % 8
                        pieces.append(zero8f if r == 7 else pltpu.unpack_elementwise(
                            kn[r, pl.ds(7 * j, 8), :], index=pair, packed_dtype=BF16,
                            unpacked_dtype=F32))
                    kk = jnp.concatenate(pieces, axis=0).astype(BF16)
                    sc = jnp.dot(kk, pltpu.bitcast(rq, BF16), preferred_element_type=F32)
                    scs[g % 2, t, pair, b] = jnp.concatenate(
                        [sc[8 * s:8 * s + 8] for s in range(8) if s != padslot], axis=0)

    def softmax_pv(g):
        for t in range(GRP_TILES[g]):
            padslot = (t + 7) % 8
            for pair in range(2):
                ps, ls_ = [], []
                for b in range(2):
                    sc = jnp.where(kvalid, scs[g % 2, t, pair, b], -jnp.inf)
                    m = jnp.max(sc, axis=0, keepdims=True)
                    p = jnp.exp2(sc - m)
                    ls_.append(jnp.sum(p, axis=0, keepdims=True))
                    blocks, k = [], 0
                    for s in range(8):
                        if s == padslot:
                            blocks.append(zero8f)
                        else:
                            blocks.append(p[8 * k:8 * k + 8])
                            k += 1
                    ps.append(jnp.concatenate(blocks, axis=0))
                for hh in range(2):
                    if hh == 0:
                        pa = jnp.where(lo, ps[0], 0.0)
                        pb = jnp.where(lo, 0.0, ps[1])
                        l = jnp.where(lo, ls_[0], ls_[1])
                    else:
                        pa = jnp.where(lo, 0.0, ps[0])
                        pb = jnp.where(lo, ps[1], 0.0)
                        l = jnp.where(lo, ls_[1], ls_[0])
                    pfull = jnp.concatenate([pa, pb], axis=0).astype(BF16)
                    hrow = pl.ds(_hpos(2 * pair + hh), 24)
                    v = pltpu.bitcast(dv[g, t, hrow, :], BF16)
                    o = jnp.dot(v, pfull, preferred_element_type=F32)
                    rl = pltpu.reciprocal(l, approx=True)
                    rl = rl * (2.0 - l * rl)
                    o = o * rl
                    do[g, t, hrow, :] = pltpu.pack_elementwise(
                        [o[:24], o[24:]], packed_dtype=BF16)

    def inverse(g):
        for hd in range(NH):
            rs = pl.ds(24 * hd, 24)
            ins = [do[g, t, rs, :] if t < GRP_TILES[g] else zero24 for t in range(8)]
            for r, v in enumerate(_barrel(ins, masks, WS)):
                ob[g, r, rs, :] = v
        for r in range(WS):
            for par in range(2):
                rows = pl.ds(48 * par, 48)
                idx = jnp.concatenate([pat_ref[_pidx(1, g, r, par)]] * 6, axis=0)
                res[r, g, rows, :] = jnp.take_along_axis(ob[g, r, rows, :], idx, axis=1)

    def out_proj(rows):
        bounds = (112, 96, 80, 64)
        for r in rows:
            tiles = [jnp.where(lane1 < bounds[s], res[r, s], res[r, s + 1]) for s in range(4)]
            oimg = pltpu.bitcast(jnp.concatenate(tiles, axis=1), BF16)
            y = jnp.dot(wos[...], oimg, preferred_element_type=F32)
            o_ref[r] = (y + x0s[r]).astype(o_ref.dtype)

    for g in range(NG):
        regroup(gq, dq, g)
    for g in range(NG):
        regroup(gv, dv, g)
    block(lambda: scores(0))
    for g in range(NG):
        def stage_b(g=g):
            if g + 1 < NG:
                scores(g + 1)
            softmax_pv(g)
        block(stage_b)
    for g in range(NG):
        inverse(g)
    out_proj(range(WS))


@jax.jit
def pallas_standalone__window_attn_davit__vision_kernel(x, dw_pe, w_qkv, w_o):
    B, Hh, Ww, Cc = x.shape
    assert (B, Hh, Ww, Cc) == (1, H, W, C)
    xt = jnp.transpose(x, (0, 1, 3, 2)).reshape(H, C, W)
    dwb = jnp.broadcast_to(dw_pe.reshape(9, C, 1), (9, C, 128))
    wt = jnp.transpose(w_qkv)
    wo = jnp.transpose(w_o)
    pat = jnp.asarray(_pattern_table())

    def row_spec(k):
        return pl.BlockSpec((1, C, WP), lambda i: (jnp.minimum(WS * i + 3 + k, H - 1), 0, 0))

    out = pl.pallas_call(
        _kernel,
        grid=(NSTRIP,),
        in_specs=[
            pl.BlockSpec((1, C, WP), lambda i: (0, 0, 0)),
            pl.BlockSpec((1, C, WP), lambda i: (1, 0, 0)),
            pl.BlockSpec((1, C, WP), lambda i: (2, 0, 0)),
            *[row_spec(k) for k in range(WS)],
            pl.BlockSpec((9, C, 128), lambda i: (0, 0, 0)),
            pl.BlockSpec((3 * C, C), lambda i: (0, 0)),
            pl.BlockSpec((C, C), lambda i: (0, 0)),
            pl.BlockSpec(pat.shape, lambda i: (0, 0, 0)),
        ],
        out_specs=pl.BlockSpec((WS, C, WP), lambda i: (i, 0, 0)),
        out_shape=jax.ShapeDtypeStruct((H, C, W), x.dtype),
        scratch_shapes=[
            pltpu.VMEM((9, C, 128), F32),
            pltpu.VMEM((3 * C, C), BF16),
            pltpu.VMEM((C, C), BF16),
            pltpu.VMEM((WS, C, WP), F32),
            pltpu.VMEM((2, C, WP), F32),
            pltpu.VMEM((2, C, WP), F32),
            pltpu.VMEM((WS, C // 2, WP), U32),
            pltpu.VMEM((WS, NG, 96, 128), U32),
            pltpu.VMEM((WS, NG, 96, 128), U32),
            pltpu.VMEM((WS, WP, 128), U32),
            pltpu.VMEM((NG, 8, 96, 128), U32),
            pltpu.VMEM((NG, 8, 96, 128), U32),
            pltpu.VMEM((NG, 8, 96, 128), U32),
            pltpu.VMEM((2, 8, 2, 2, 56, 128), F32),
            pltpu.VMEM((WS, NG, 96, 128), U32),
            pltpu.VMEM((NG, WS, 96, 128), U32),
        ],
        compiler_params=pltpu.CompilerParams(
            dimension_semantics=("arbitrary",),
            vmem_limit_bytes=100 * 1024 * 1024,
        ),
    )(*([xt] * (WS + 3)), dwb, wt, wo, pat)
    return jnp.transpose(out.reshape(1, H, C, W), (0, 1, 3, 2))
```

```python
import numpy as np
import jax
import jax.numpy as jnp
from jax import lax
import jax.experimental.pallas as pl
import jax.experimental.pallas.tpu as pltpu

WS = 7
NH = 4
C = 192
DH = C // NH
H = W = 511
WP = 512
NSTRIP = H // WS
NWIN = W // WS
NG = 5
GRP_TILES = (8, 8, 8, 8, 5)
LOG2E = 1.4426950408889634
EPS = 1e-5
U32 = jnp.uint32
F32 = jnp.float32
BF16 = jnp.bfloat16


def _fwd_pattern(g, r, par):
    lane = np.arange(128)
    bp, s, c = lane // 64, (lane // 8) % 8, lane % 8
    b = bp ^ par
    t = (s - r) % 8
    jj = 2 * t + b
    return ((112 * g + 7 * jj + np.minimum(c, 6)) % 128).astype(np.int32)


def _inv_pattern(g, r, par):
    idx = np.zeros(128, np.int32)
    for jj in range(16):
        t, b = jj // 2, jj % 2
        for c in range(7):
            p = (112 * g + 7 * jj + c) % 128
            idx[p] = 64 * (b ^ par) + 8 * ((t + r) % 8) + c
    return idx


def _pattern_table():
    rows = []
    for g in range(NG):
        for r in range(WS):
            for par in range(2):
                rows.append(_fwd_pattern(g, r, par))
    for g in range(NG):
        for r in range(WS):
            for par in range(2):
                rows.append(_inv_pattern(g, r, par))
    tab = np.stack(rows)
    return np.broadcast_to(tab[:, None, :], (tab.shape[0], 8, 128)).copy()


def _pidx(inv, g, r, par):
    return ((inv * NG + g) * WS + r) * 2 + par


def _hpos(hd):
    return 48 * (hd % 2) + 24 * (hd // 2)


def _barrel(ins, masks, nout):
    m1, m2, m4 = masks
    u = [ins[(-m) % 8] for m in range(8)]
    v1 = [jnp.where(m1, u[(t - 1) % 8], u[t]) for t in range(8)]
    v2 = [jnp.where(m2, v1[(t - 2) % 8], v1[t]) for t in range(8)]
    return [jnp.where(m4, v2[(t - 4) % 8], v2[t]) for t in range(nout)]


def _kernel(x0_ref, x1_ref, x2_ref, xa_ref, xb_ref, xc_ref, xd_ref, xe_ref, xf_ref, xg_ref,
            dw_ref, wt_ref, wo_ref, pat_ref, o_ref,
            wtab, wts, wos, x0s, xcs, x0n, hs_a, hs_b, hs_c, gq, gv, kn, dq, dv, do, scs_a, scs_b, res, ob):
    i = pl.program_id(0)
    one = jnp.where(i >= 0, 1, 0)
    hs = (hs_a, hs_b, hs_a, hs_b, hs_a, hs_b, hs_c)
    scs = (scs_a, scs_b)
    xrows = (xa_ref, xb_ref, xc_ref, xd_ref, xe_ref, xf_ref, xg_ref)

    lane1 = lax.broadcasted_iota(jnp.int32, (1, 128), 1)
    lane512 = lax.broadcasted_iota(jnp.int32, (1, WP), 1)

    def block(fn):
        lax.fori_loop(0, one, lambda _, c: (fn(), c)[1], 0)

    def conv_row(x_ref, valid, taps):
        for ch in range(12):
            rs = pl.ds(16 * ch, 16)
            xp = pltpu.bitcast(x_ref[0, rs, :], U32)
            if valid is None:
                last = jnp.where(lane1 < W - 384, xp[:, 384:], jnp.zeros_like(xp[:, 384:]))
                xp = jnp.concatenate([xp[:, :384], last], axis=1)
            else:
                xp = jnp.where((lane512 < W) & valid, xp, jnp.zeros_like(xp))
            xl = pltpu.roll(xp, 1, 1)
            first = jnp.where(lane1 > 0, xl[:, :128], jnp.zeros_like(xl[:, :128]))
            xl = jnp.concatenate([first, xl[:, 128:]], axis=1)
            xr = pltpu.roll(xp, WP - 1, 1)
            ws = [wtab[k, rs, :] for k in range(9)]
            for s_ in range(4):
                ls = pl.ds(128 * s_, 128)
                xs = [pltpu.bitcast(v[:, 128 * s_:128 * (s_ + 1)], BF16).astype(F32)
                      for v in (xl, xp, xr)]
                for ki, tap in enumerate(taps):
                    if tap is None:
                        continue
                    dst, src = tap
                    t = xs[0] * ws[3 * ki] + xs[1] * ws[3 * ki + 1] + xs[2] * ws[3 * ki + 2]
                    dst[rs, ls] = t if src is None else src[rs, ls] + t

    def layer_norm(x0_row, q):
        for s in range(4):
            ls = pl.ds(128 * s, 128)
            x0 = x0_row[:, ls]
            mean = jnp.sum(x0, axis=0, keepdims=True) * (1.0 / C)
            xc = x0 - mean
            var = jnp.sum(xc * xc, axis=0, keepdims=True) * (1.0 / C)
            hn = xc * lax.rsqrt(var + EPS)
            hs[q][:, ls] = pltpu.pack_elementwise([hn[:96], hn[96:]], packed_dtype=BF16)

    @pl.when(i == 0)
    def _init():
        for k in range(9):
            w = dw_ref[k].astype(F32)
            if k == 4:
                w = w + 1.0
            wtab[k] = w
        src = lax.broadcasted_iota(jnp.int32, (C, C), 0)
        pos = lax.broadcasted_iota(jnp.int32, (C, C), 1)
        p_chan = (src == (pos >> 1) + 96 * (pos & 1)).astype(BF16)
        hp, within = pos // DH, pos % DH
        hd = 2 * (hp % 2) + hp // 2
        p_head = (src == hd * DH + (within >> 1) + 24 * (within & 1)).astype(BF16)
        wt = jnp.dot(wt_ref[...], p_chan, preferred_element_type=F32).astype(BF16)
        r_in, r_hp = src % DH, src // DH
        r_hd = 2 * (r_hp % 2) + r_hp // 2
        p_rows = (pos == r_hd * DH + 2 * (r_in % 24) + r_in // 24).astype(BF16)
        wq = jnp.dot(p_rows, wt[0:C], preferred_element_type=F32)
        wts[0:C, :] = (wq * (DH ** -0.5 * LOG2E)).astype(BF16)
        wts[C:2 * C, :] = wt[C:2 * C]
        wts[2 * C:3 * C, :] = jnp.dot(p_rows, wt[2 * C:3 * C],
                                      preferred_element_type=F32).astype(BF16)
        wos[...] = jnp.dot(wo_ref[...], p_head, preferred_element_type=F32).astype(BF16)
        n0, n1, c0, c1 = x0n.at[0], x0n.at[1], xcs.at[0], xcs.at[1]
        conv_row(x0_ref, None, ((n1, None), (n0, None), None))
        conv_row(x1_ref, None, ((c0, None), (n1, n1), (n0, n0)))
        conv_row(x2_ref, None, ((c1, None), (c0, c0), (n1, n1)))
        layer_norm(n0, 0)

    offs = [((112 * g) // 128, (112 * g) % 128) for g in range(NG)]

    def gather_qv(yh, dst, r, rows, par):
        for g in range(NG):
            a, off = offs[g]
            src = yh[:, 128 * a:128 * (a + 1)]
            if g not in (0, NG - 1):
                src = jnp.where(lane1 >= off, src, yh[:, 128 * (a + 1):128 * (a + 2)])
            idx = jnp.concatenate([pat_ref[_pidx(0, g, r, par)]] * 6, axis=0)
            dst[r, g, rows, :] = jnp.take_along_axis(src, idx, axis=1)

    def qkv_row(r):
        h = pltpu.bitcast(hs[r][...], BF16)
        for s in range(4):
            yk = jnp.dot(wts[C:2 * C, :], h[:, 128 * s:128 * (s + 1)], preferred_element_type=F32)
            kp = pltpu.pack_elementwise([yk[:96], yk[96:]], packed_dtype=BF16)
            blk = jnp.concatenate([kp, jnp.zeros((32, 128), U32)], axis=0)
            kn[r, pl.ds(128 * s, 128), :] = blk.T
        for base, dst in ((0, gq), (2 * C, gv)):
            y2 = jnp.dot(wts[pl.ds(base, C), :], h, preferred_element_type=F32)
            for cls in range(2):
                y = y2[96 * cls:96 * cls + 96]
                yh = jnp.concatenate([
                    pltpu.pack_elementwise([y[48 * hh:48 * hh + 24], y[48 * hh + 24:48 * hh + 48]],
                                           packed_dtype=BF16) for hh in range(2)], axis=0)
                gather_qv(yh, dst, r, pl.ds(48 * cls, 48), cls if base == 0 else 0)

    def part(q):
        if 4 <= q <= 6:
            return x0s.at[q]
        return x0n.at[q - 7] if q in (7, 8) else xcs.at[(q - 2) % WS]

    def final(q):
        if 2 <= q <= 6:
            return x0s.at[q]
        return x0n.at[q % WS]

    for r in range(WS):
        def stage_a(r=r):
            valid = None if r < 4 else (WS * i + 3 + r < H)
            qkv_row(r)
            layer_norm(final(r + 1), (r + 1) % WS)
            if r < 2:
                x0s[r] = x0n[r]
            conv_row(xrows[r], valid, ((part(r + 4), None), (part(r + 3), part(r + 3)),
                                       (final(r + 2), part(r + 2))))
        stage_a()

    masks = (((lane1 >> 3) & 1) == 1, ((lane1 >> 4) & 1) == 1, ((lane1 >> 5) & 1) == 1)
    zero8 = jnp.zeros((8, 128), U32)
    zero24 = jnp.zeros((24, 128), U32)
    zero16 = jnp.zeros((16, 128), U32)
    zero8f = jnp.zeros((8, 128), F32)
    lo = lane1 < 64
    kvalid = (lax.broadcasted_iota(jnp.int32, (56, 128), 0) & 7) < 7

    def regroup(src, dst, g):
        for k in range(12):
            rs = pl.ds(8 * k, 8)
            ins = [src[r, g, rs, :] for r in range(WS)] + [zero8]
            for t, v in enumerate(_barrel(ins, masks, GRP_TILES[g])):
                dst[g, t, rs, :] = v

    def scores(g):
        for t in range(GRP_TILES[g]):
            padslot = (t + 7) % 8
            for pair in range(2):
                qe = dq[g, t, pl.ds(_hpos(2 * pair), 24), :]
                qo = dq[g, t, pl.ds(_hpos(2 * pair + 1), 24), :]
                ra = jnp.concatenate(
                    [jnp.where(lo, qe, zero24), jnp.where(lo, zero24, qo), zero16], axis=0)
                rb = jnp.concatenate(
                    [jnp.where(lo, zero24, qe), jnp.where(lo, qo, zero24), zero16], axis=0)
                for b, rq in ((0, ra), (1, rb)):
                    j = min(16 * g + 2 * t + b, NWIN - 1)
                    pieces = []
                    for s in range(8):
                        r = (s - t) % 8
                        pieces.append(zero8f if r == 7 else pltpu.unpack_elementwise(
                            kn[r, pl.ds(7 * j, 8), :], index=pair, packed_dtype=BF16,
                            unpacked_dtype=F32))
                    kk = jnp.concatenate(pieces, axis=0).astype(BF16)
                    sc = jnp.dot(kk, pltpu.bitcast(rq, BF16), preferred_element_type=F32)
                    scs[g % 2][t, pair, b] = jnp.concatenate(
                        [sc[8 * s:8 * s + 8] for s in range(8) if s != padslot], axis=0)

    def softmax_pv(g):
        for t in range(GRP_TILES[g]):
            padslot = (t + 7) % 8
            for pair in range(2):
                ps, ls_ = [], []
                for b in range(2):
                    sc = jnp.where(kvalid, scs[g % 2][t, pair, b], -jnp.inf)
                    m = jnp.max(sc, axis=0, keepdims=True)
                    p = jnp.exp2(sc - m)
                    ls_.append(jnp.sum(p, axis=0, keepdims=True))
                    blocks, k = [], 0
                    for s in range(8):
                        if s == padslot:
                            blocks.append(zero8f)
                        else:
                            blocks.append(p[8 * k:8 * k + 8])
                            k += 1
                    ps.append(jnp.concatenate(blocks, axis=0))
                for hh in range(2):
                    if hh == 0:
                        pa = jnp.where(lo, ps[0], 0.0)
                        pb = jnp.where(lo, 0.0, ps[1])
                        l = jnp.where(lo, ls_[0], ls_[1])
                    else:
                        pa = jnp.where(lo, 0.0, ps[0])
                        pb = jnp.where(lo, ps[1], 0.0)
                        l = jnp.where(lo, ls_[1], ls_[0])
                    pfull = jnp.concatenate([pa, pb], axis=0).astype(BF16)
                    hrow = pl.ds(_hpos(2 * pair + hh), 24)
                    v = pltpu.bitcast(dv[g, t, hrow, :], BF16)
                    o = jnp.dot(v, pfull, preferred_element_type=F32)
                    rl = pltpu.reciprocal(l, approx=True)
                    rl = rl * (2.0 - l * rl)
                    o = o * rl
                    do[g, t, hrow, :] = pltpu.pack_elementwise(
                        [o[:24], o[24:]], packed_dtype=BF16)

    def inverse(g):
        for k in range(12):
            rs = pl.ds(8 * k, 8)
            ins = [do[g, t, rs, :] if t < GRP_TILES[g] else zero8 for t in range(8)]
            for r, v in enumerate(_barrel(ins, masks, WS)):
                ob[g, r, rs, :] = v
        for r in range(WS):
            for par in range(2):
                rows = pl.ds(48 * par, 48)
                idx = jnp.concatenate([pat_ref[_pidx(1, g, r, par)]] * 6, axis=0)
                res[r, g, rows, :] = jnp.take_along_axis(ob[g, r, rows, :], idx, axis=1)

    def out_proj(rows):
        bounds = (112, 96, 80, 64)
        for r in rows:
            tiles = [jnp.where(lane1 < bounds[s], res[r, s], res[r, s + 1]) for s in range(4)]
            oimg = pltpu.bitcast(jnp.concatenate(tiles, axis=1), BF16)
            y = jnp.dot(wos[...], oimg, preferred_element_type=F32)
            o_ref[r] = (y + x0s[r]).astype(o_ref.dtype)

    for g in range(NG):
        regroup(gq, dq, g)
    for g in range(NG):
        regroup(gv, dv, g)
    block(lambda: scores(0))
    for g in range(NG):
        def stage_b(g=g):
            if g + 1 < NG:
                scores(g + 1)
            softmax_pv(g)
        block(stage_b)
    for g in range(NG):
        inverse(g)
    out_proj(range(WS))


@jax.jit
def pallas_standalone__window_attn_davit__vision_kernel(x, dw_pe, w_qkv, w_o):
    B, Hh, Ww, Cc = x.shape
    assert (B, Hh, Ww, Cc) == (1, H, W, C)
    xt = jnp.transpose(x, (0, 1, 3, 2)).reshape(H, C, W)
    dwb = jnp.broadcast_to(dw_pe.reshape(9, C, 1), (9, C, 128))
    wt = jnp.transpose(w_qkv)
    wo = jnp.transpose(w_o)
    pat = jnp.asarray(_pattern_table())

    def row_spec(k):
        return pl.BlockSpec((1, C, WP), lambda i: (jnp.minimum(WS * i + 3 + k, H - 1), 0, 0))

    out = pl.pallas_call(
        _kernel,
        grid=(NSTRIP,),
        in_specs=[
            pl.BlockSpec((1, C, WP), lambda i: (0, 0, 0)),
            pl.BlockSpec((1, C, WP), lambda i: (1, 0, 0)),
            pl.BlockSpec((1, C, WP), lambda i: (2, 0, 0)),
            *[row_spec(k) for k in range(WS)],
            pl.BlockSpec((9, C, 128), lambda i: (0, 0, 0)),
            pl.BlockSpec((3 * C, C), lambda i: (0, 0)),
            pl.BlockSpec((C, C), lambda i: (0, 0)),
            pl.BlockSpec(pat.shape, lambda i: (0, 0, 0)),
        ],
        out_specs=pl.BlockSpec((WS, C, WP), lambda i: (i, 0, 0)),
        out_shape=jax.ShapeDtypeStruct((H, C, W), x.dtype),
        scratch_shapes=[
            pltpu.VMEM((9, C, 128), F32),
            pltpu.VMEM((3 * C, C), BF16),
            pltpu.VMEM((C, C), BF16),
            pltpu.VMEM((WS, C, WP), F32),
            pltpu.VMEM((2, C, WP), F32),
            pltpu.VMEM((2, C, WP), F32),
            *[pltpu.VMEM((C // 2, WP), U32)] * 3,
            pltpu.VMEM((WS, NG, 96, 128), U32),
            pltpu.VMEM((WS, NG, 96, 128), U32),
            pltpu.VMEM((WS, WP, 128), U32),
            pltpu.VMEM((NG, 8, 96, 128), U32),
            pltpu.VMEM((NG, 8, 96, 128), U32),
            pltpu.VMEM((NG, 8, 96, 128), U32),
            *[pltpu.VMEM((8, 2, 2, 56, 128), F32)] * 2,
            pltpu.VMEM((WS, NG, 96, 128), U32),
            pltpu.VMEM((NG, WS, 96, 128), U32),
        ],
        compiler_params=pltpu.CompilerParams(
            dimension_semantics=("arbitrary",),
            vmem_limit_bytes=100 * 1024 * 1024,
        ),
    )(*([xt] * (WS + 3)), dwb, wt, wo, pat)
    return jnp.transpose(out.reshape(1, H, C, W), (0, 1, 3, 2))
```

```python
import numpy as np
import jax
import jax.numpy as jnp
from jax import lax
import jax.experimental.pallas as pl
import jax.experimental.pallas.tpu as pltpu

WS = 7
NH = 4
C = 192
DH = C // NH
H = W = 511
WP = 512
NSTRIP = H // WS
NWIN = W // WS
NG = 5
GRP_TILES = (8, 8, 8, 8, 5)
LOG2E = 1.4426950408889634
EPS = 1e-5
U32 = jnp.uint32
F32 = jnp.float32
BF16 = jnp.bfloat16


def _fwd_pattern(g, r, par):
    lane = np.arange(128)
    bp, s, c = lane // 64, (lane // 8) % 8, lane % 8
    b = bp ^ par
    t = (s - r) % 8
    jj = 2 * t + b
    return ((112 * g + 7 * jj + np.minimum(c, 6)) % 128).astype(np.int32)


def _inv_pattern(g, r, par):
    idx = np.zeros(128, np.int32)
    for jj in range(16):
        t, b = jj // 2, jj % 2
        for c in range(7):
            p = (112 * g + 7 * jj + c) % 128
            idx[p] = 64 * (b ^ par) + 8 * ((t + r) % 8) + c
    return idx


def _pattern_table():
    rows = []
    for g in range(NG):
        for r in range(WS):
            for par in range(2):
                rows.append(_fwd_pattern(g, r, par))
    for g in range(NG):
        for r in range(WS):
            for par in range(2):
                rows.append(_inv_pattern(g, r, par))
    tab = np.stack(rows)
    return np.broadcast_to(tab[:, None, :], (tab.shape[0], 8, 128)).copy()


def _pidx(inv, g, r, par):
    return ((inv * NG + g) * WS + r) * 2 + par


def _hpos(hd):
    return 48 * (hd % 2) + 24 * (hd // 2)


def _barrel(ins, masks, nout):
    m1, m2, m4 = masks
    u = [ins[(-m) % 8] for m in range(8)]
    v1 = [jnp.where(m1, u[(t - 1) % 8], u[t]) for t in range(8)]
    v2 = [jnp.where(m2, v1[(t - 2) % 8], v1[t]) for t in range(8)]
    return [jnp.where(m4, v2[(t - 4) % 8], v2[t]) for t in range(nout)]


def _kernel(x0_ref, x1_ref, x2_ref, xa_ref, xb_ref, xc_ref, xd_ref, xe_ref, xf_ref, xg_ref,
            dw_ref, wt_ref, wo_ref, pat_ref, o_ref,
            wtab, wts, wos, x0s, xcs, x0n, hs_a, hs_b, hs_c, gq, gv, kn, dq, dv, do, scs_a, scs_b, res, ob):
    i = pl.program_id(0)
    one = jnp.where(i >= 0, 1, 0)
    hs = (hs_a, hs_b, hs_a, hs_b, hs_a, hs_b, hs_c)
    scs = (scs_a, scs_b)
    xrows = (xa_ref, xb_ref, xc_ref, xd_ref, xe_ref, xf_ref, xg_ref)

    lane1 = lax.broadcasted_iota(jnp.int32, (1, 128), 1)
    lane512 = lax.broadcasted_iota(jnp.int32, (1, WP), 1)

    def block(fn):
        lax.fori_loop(0, one, lambda _, c: (fn(), c)[1], 0)

    def conv_row(x_ref, valid, taps):
        for ch in range(12):
            rs = pl.ds(16 * ch, 16)
            xp = pltpu.bitcast(x_ref[0, rs, :], U32)
            if valid is None:
                last = jnp.where(lane1 < W - 384, xp[:, 384:], jnp.zeros_like(xp[:, 384:]))
                xp = jnp.concatenate([xp[:, :384], last], axis=1)
            else:
                xp = jnp.where((lane512 < W) & valid, xp, jnp.zeros_like(xp))
            xl = pltpu.roll(xp, 1, 1)
            first = jnp.where(lane1 > 0, xl[:, :128], jnp.zeros_like(xl[:, :128]))
            xl = jnp.concatenate([first, xl[:, 128:]], axis=1)
            xr = pltpu.roll(xp, WP - 1, 1)
            ws = [wtab[k, rs, :] for k in range(9)]
            for s_ in range(4):
                ls = pl.ds(128 * s_, 128)
                xs = [pltpu.bitcast(v[:, 128 * s_:128 * (s_ + 1)], BF16).astype(F32)
                      for v in (xl, xp, xr)]
                for ki, tap in enumerate(taps):
                    if tap is None:
                        continue
                    dst, src = tap
                    t = xs[0] * ws[3 * ki] + xs[1] * ws[3 * ki + 1] + xs[2] * ws[3 * ki + 2]
                    dst[rs, ls] = t if src is None else src[rs, ls] + t

    def layer_norm(x0_row, q):
        for s in range(4):
            ls = pl.ds(128 * s, 128)
            x0 = x0_row[:, ls]
            mean = jnp.sum(x0, axis=0, keepdims=True) * (1.0 / C)
            xc = x0 - mean
            var = jnp.sum(xc * xc, axis=0, keepdims=True) * (1.0 / C)
            hn = xc * lax.rsqrt(var + EPS)
            hs[q][:, ls] = pltpu.pack_elementwise([hn[:96], hn[96:]], packed_dtype=BF16)

    @pl.when(i == 0)
    def _init():
        for k in range(9):
            w = dw_ref[k].astype(F32)
            if k == 4:
                w = w + 1.0
            wtab[k] = w
        src = lax.broadcasted_iota(jnp.int32, (C, C), 0)
        pos = lax.broadcasted_iota(jnp.int32, (C, C), 1)
        p_chan = (src == (pos >> 1) + 96 * (pos & 1)).astype(BF16)
        hp, within = pos // DH, pos % DH
        hd = 2 * (hp % 2) + hp // 2
        p_head = (src == hd * DH + (within >> 1) + 24 * (within & 1)).astype(BF16)
        wt = jnp.dot(wt_ref[...], p_chan, preferred_element_type=F32).astype(BF16)
        r_in, r_hp = src % DH, src // DH
        r_hd = 2 * (r_hp % 2) + r_hp // 2
        p_rows = (pos == r_hd * DH + 2 * (r_in % 24) + r_in // 24).astype(BF16)
        wq = jnp.dot(p_rows, wt[0:C], preferred_element_type=F32)
        wts[0:C, :] = (wq * (DH ** -0.5 * LOG2E)).astype(BF16)
        wts[C:2 * C, :] = wt[C:2 * C]
        wts[2 * C:3 * C, :] = jnp.dot(p_rows, wt[2 * C:3 * C],
                                      preferred_element_type=F32).astype(BF16)
        wos[...] = jnp.dot(wo_ref[...], p_head, preferred_element_type=F32).astype(BF16)
        n0, n1, c0, c1 = x0n.at[0], x0n.at[1], xcs.at[0], xcs.at[1]
        conv_row(x0_ref, None, ((n1, None), (n0, None), None))
        conv_row(x1_ref, None, ((c0, None), (n1, n1), (n0, n0)))
        conv_row(x2_ref, None, ((c1, None), (c0, c0), (n1, n1)))
        layer_norm(n0, 0)

    offs = [((112 * g) // 128, (112 * g) % 128) for g in range(NG)]

    def gather_qv(yh, dst, r, rows, par):
        for g in range(NG):
            a, off = offs[g]
            src = yh[:, 128 * a:128 * (a + 1)]
            if g not in (0, NG - 1):
                src = jnp.where(lane1 >= off, src, yh[:, 128 * (a + 1):128 * (a + 2)])
            idx = jnp.concatenate([pat_ref[_pidx(0, g, r, par)]] * 6, axis=0)
            dst[r, g, rows, :] = jnp.take_along_axis(src, idx, axis=1)

    def qkv_row(r):
        h = pltpu.bitcast(hs[r][...], BF16)
        for s in range(4):
            yk = jnp.dot(wts[C:2 * C, :], h[:, 128 * s:128 * (s + 1)], preferred_element_type=F32)
            kp = pltpu.pack_elementwise([yk[:96], yk[96:]], packed_dtype=BF16)
            blk = jnp.concatenate([kp, jnp.zeros((32, 128), U32)], axis=0)
            kn[r, pl.ds(128 * s, 128), :] = blk.T
        for base, dst in ((0, gq), (2 * C, gv)):
            y2 = jnp.dot(wts[pl.ds(base, C), :], h, preferred_element_type=F32)
            for cls in range(2):
                y = y2[96 * cls:96 * cls + 96]
                yh = jnp.concatenate([
                    pltpu.pack_elementwise([y[48 * hh:48 * hh + 24], y[48 * hh + 24:48 * hh + 48]],
                                           packed_dtype=BF16) for hh in range(2)], axis=0)
                gather_qv(yh, dst, r, pl.ds(48 * cls, 48), cls if base == 0 else 0)

    def part(q):
        if 4 <= q <= 6:
            return x0s.at[q]
        return x0n.at[q - 7] if q in (7, 8) else xcs.at[(q - 2) % WS]

    def final(q):
        if 2 <= q <= 6:
            return x0s.at[q]
        return x0n.at[q % WS]

    for r in range(WS):
        def stage_a(r=r):
            valid = None if r < 4 else (WS * i + 3 + r < H)
            qkv_row(r)
            layer_norm(final(r + 1), (r + 1) % WS)
            if r < 2:
                x0s[r] = x0n[r]
            conv_row(xrows[r], valid, ((part(r + 4), None), (part(r + 3), part(r + 3)),
                                       (final(r + 2), part(r + 2))))
        stage_a()

    masks = (((lane1 >> 3) & 1) == 1, ((lane1 >> 4) & 1) == 1, ((lane1 >> 5) & 1) == 1)
    zero8 = jnp.zeros((8, 128), U32)
    zero24 = jnp.zeros((24, 128), U32)
    zero16 = jnp.zeros((16, 128), U32)
    zero8f = jnp.zeros((8, 128), F32)
    lo = lane1 < 64
    kvalid = (lax.broadcasted_iota(jnp.int32, (56, 128), 0) & 7) < 7

    def regroup(src, dst, g):
        for k in range(12):
            rs = pl.ds(8 * k, 8)
            ins = [src[r, g, rs, :] for r in range(WS)] + [zero8]
            for t, v in enumerate(_barrel(ins, masks, GRP_TILES[g])):
                dst[g, t, rs, :] = v

    def scores(g):
        for t in range(GRP_TILES[g]):
            padslot = (t + 7) % 8
            for pair in range(2):
                qe = dq[g, t, pl.ds(_hpos(2 * pair), 24), :]
                qo = dq[g, t, pl.ds(_hpos(2 * pair + 1), 24), :]
                ra = jnp.concatenate(
                    [jnp.where(lo, qe, zero24), jnp.where(lo, zero24, qo), zero16], axis=0)
                rb = jnp.concatenate(
                    [jnp.where(lo, zero24, qe), jnp.where(lo, qo, zero24), zero16], axis=0)
                for b, rq in ((0, ra), (1, rb)):
                    j = min(16 * g + 2 * t + b, NWIN - 1)
                    pieces = []
                    for s in range(8):
                        r = (s - t) % 8
                        pieces.append(zero8f if r == 7 else pltpu.unpack_elementwise(
                            kn[r, pl.ds(7 * j, 8), :], index=pair, packed_dtype=BF16,
                            unpacked_dtype=F32))
                    kk = jnp.concatenate(pieces, axis=0).astype(BF16)
                    sc = jnp.dot(kk, pltpu.bitcast(rq, BF16), preferred_element_type=F32)
                    scs[g % 2][t, pair, b] = jnp.concatenate(
                        [sc[8 * s:8 * s + 8] for s in range(8) if s != padslot], axis=0)

    def softmax_pv(g):
        for t in range(GRP_TILES[g]):
            padslot = (t + 7) % 8
            for pair in range(2):
                ps, ls_ = [], []
                for b in range(2):
                    sc = jnp.where(kvalid, scs[g % 2][t, pair, b], -jnp.inf)
                    m = jnp.max(sc, axis=0, keepdims=True)
                    p = jnp.exp2(sc - m)
                    ls_.append(jnp.sum(p, axis=0, keepdims=True))
                    blocks, k = [], 0
                    for s in range(8):
                        if s == padslot:
                            blocks.append(zero8f)
                        else:
                            blocks.append(p[8 * k:8 * k + 8])
                            k += 1
                    ps.append(jnp.concatenate(blocks, axis=0))
                for hh in range(2):
                    if hh == 0:
                        pa = jnp.where(lo, ps[0], 0.0)
                        pb = jnp.where(lo, 0.0, ps[1])
                        l = jnp.where(lo, ls_[0], ls_[1])
                    else:
                        pa = jnp.where(lo, 0.0, ps[0])
                        pb = jnp.where(lo, ps[1], 0.0)
                        l = jnp.where(lo, ls_[1], ls_[0])
                    pfull = jnp.concatenate([pa, pb], axis=0).astype(BF16)
                    hrow = pl.ds(_hpos(2 * pair + hh), 24)
                    v = pltpu.bitcast(dv[g, t, hrow, :], BF16)
                    o = jnp.dot(v, pfull, preferred_element_type=F32)
                    rl = pltpu.reciprocal(l, approx=True)
                    rl = rl * (2.0 - l * rl)
                    o = o * rl
                    do[g, t, hrow, :] = pltpu.pack_elementwise(
                        [o[:24], o[24:]], packed_dtype=BF16)

    def inverse(g):
        for k in range(12):
            rs = pl.ds(8 * k, 8)
            ins = [do[g, t, rs, :] if t < GRP_TILES[g] else zero8 for t in range(8)]
            for r, v in enumerate(_barrel(ins, masks, WS)):
                ob[g, r, rs, :] = v
        for r in range(WS):
            for par in range(2):
                rows = pl.ds(48 * par, 48)
                idx = jnp.concatenate([pat_ref[_pidx(1, g, r, par)]] * 6, axis=0)
                res[r, g, rows, :] = jnp.take_along_axis(ob[g, r, rows, :], idx, axis=1)

    def out_proj(rows):
        bounds = (112, 96, 80, 64)
        for r in rows:
            tiles = [jnp.where(lane1 < bounds[s], res[r, s], res[r, s + 1]) for s in range(4)]
            oimg = pltpu.bitcast(jnp.concatenate(tiles, axis=1), BF16)
            y = jnp.dot(wos[...], oimg, preferred_element_type=F32)
            o_ref[r] = (y + x0s[r]).astype(o_ref.dtype)

    for g in range(NG):
        regroup(gq, dq, g)
    for g in range(NG):
        regroup(gv, dv, g)
    scores(0)
    for g in range(NG):
        def stage_b(g=g):
            if g + 1 < NG:
                scores(g + 1)
            softmax_pv(g)
        if g < NG - 1:
            block(stage_b)
        else:
            stage_b()
    for g in range(NG):
        inverse(g)
    out_proj(range(WS))


@jax.jit
def pallas_standalone__window_attn_davit__vision_kernel(x, dw_pe, w_qkv, w_o):
    B, Hh, Ww, Cc = x.shape
    assert (B, Hh, Ww, Cc) == (1, H, W, C)
    xt = jnp.transpose(x, (0, 1, 3, 2)).reshape(H, C, W)
    dwb = jnp.broadcast_to(dw_pe.reshape(9, C, 1), (9, C, 128))
    wt = jnp.transpose(w_qkv)
    wo = jnp.transpose(w_o)
    pat = jnp.asarray(_pattern_table())

    def row_spec(k):
        return pl.BlockSpec((1, C, WP), lambda i: (jnp.minimum(WS * i + 3 + k, H - 1), 0, 0))

    out = pl.pallas_call(
        _kernel,
        grid=(NSTRIP,),
        in_specs=[
            pl.BlockSpec((1, C, WP), lambda i: (0, 0, 0)),
            pl.BlockSpec((1, C, WP), lambda i: (1, 0, 0)),
            pl.BlockSpec((1, C, WP), lambda i: (2, 0, 0)),
            *[row_spec(k) for k in range(WS)],
            pl.BlockSpec((9, C, 128), lambda i: (0, 0, 0)),
            pl.BlockSpec((3 * C, C), lambda i: (0, 0)),
            pl.BlockSpec((C, C), lambda i: (0, 0)),
            pl.BlockSpec(pat.shape, lambda i: (0, 0, 0)),
        ],
        out_specs=pl.BlockSpec((WS, C, WP), lambda i: (i, 0, 0)),
        out_shape=jax.ShapeDtypeStruct((H, C, W), x.dtype),
        scratch_shapes=[
            pltpu.VMEM((9, C, 128), F32),
            pltpu.VMEM((3 * C, C), BF16),
            pltpu.VMEM((C, C), BF16),
            pltpu.VMEM((WS, C, WP), F32),
            pltpu.VMEM((2, C, WP), F32),
            pltpu.VMEM((2, C, WP), F32),
            *[pltpu.VMEM((C // 2, WP), U32)] * 3,
            pltpu.VMEM((WS, NG, 96, 128), U32),
            pltpu.VMEM((WS, NG, 96, 128), U32),
            pltpu.VMEM((WS, WP, 128), U32),
            pltpu.VMEM((NG, 8, 96, 128), U32),
            pltpu.VMEM((NG, 8, 96, 128), U32),
            pltpu.VMEM((NG, 8, 96, 128), U32),
            *[pltpu.VMEM((8, 2, 2, 56, 128), F32)] * 2,
            pltpu.VMEM((WS, NG, 96, 128), U32),
            pltpu.VMEM((NG, WS, 96, 128), U32),
        ],
        compiler_params=pltpu.CompilerParams(
            dimension_semantics=("arbitrary",),
            vmem_limit_bytes=100 * 1024 * 1024,
        ),
    )(*([xt] * (WS + 3)), dwb, wt, wo, pat)
    return jnp.transpose(out.reshape(1, H, C, W), (0, 1, 3, 2))
```

```python
import numpy as np
import jax
import jax.numpy as jnp
from jax import lax
import jax.experimental.pallas as pl
import jax.experimental.pallas.tpu as pltpu

WS = 7
NH = 4
C = 192
DH = C // NH
H = W = 511
WP = 512
NSTRIP = H // WS
NWIN = W // WS
NG = 5
GRP_TILES = (8, 8, 8, 8, 5)
LOG2E = 1.4426950408889634
EPS = 1e-5
U32 = jnp.uint32
F32 = jnp.float32
BF16 = jnp.bfloat16


def _fwd_pattern(g, r, par):
    lane = np.arange(128)
    bp, s, c = lane // 64, (lane // 8) % 8, lane % 8
    b = bp ^ par
    t = (s - r) % 8
    jj = 2 * t + b
    return ((112 * g + 7 * jj + np.minimum(c, 6)) % 128).astype(np.int32)


def _inv_pattern(g, r, par):
    idx = np.zeros(128, np.int32)
    for jj in range(16):
        t, b = jj // 2, jj % 2
        for c in range(7):
            p = (112 * g + 7 * jj + c) % 128
            idx[p] = 64 * (b ^ par) + 8 * ((t + r) % 8) + c
    return idx


def _pattern_table():
    rows = []
    for g in range(NG):
        for r in range(WS):
            for par in range(2):
                rows.append(_fwd_pattern(g, r, par))
    for g in range(NG):
        for r in range(WS):
            for par in range(2):
                rows.append(_inv_pattern(g, r, par))
    tab = np.stack(rows)
    return np.broadcast_to(tab[:, None, :], (tab.shape[0], 8, 128)).copy()


def _pidx(inv, g, r, par):
    return ((inv * NG + g) * WS + r) * 2 + par


def _hpos(hd):
    return 48 * (hd % 2) + 24 * (hd // 2)


def _barrel(ins, masks, nout):
    m1, m2, m4 = masks
    u = [ins[(-m) % 8] for m in range(8)]
    v1 = [jnp.where(m1, u[(t - 1) % 8], u[t]) for t in range(8)]
    v2 = [jnp.where(m2, v1[(t - 2) % 8], v1[t]) for t in range(8)]
    return [jnp.where(m4, v2[(t - 4) % 8], v2[t]) for t in range(nout)]


def _kernel(x0_ref, x1_ref, x2_ref, xa_ref, xb_ref, xc_ref, xd_ref, xe_ref, xf_ref, xg_ref,
            dw_ref, wt_ref, wo_ref, pat_ref, o_ref,
            wtab, wts, wos, x0s, xcs, x0n, hs_a, hs_b, hs_c, gq, gv, kn, dq, dv, do, scs_a, scs_b, res, ob):
    i = pl.program_id(0)
    one = jnp.where(i >= 0, 1, 0)
    hs = (hs_a, hs_b, hs_a, hs_b, hs_a, hs_b, hs_c)
    scs = (scs_a, scs_b)
    xrows = (xa_ref, xb_ref, xc_ref, xd_ref, xe_ref, xf_ref, xg_ref)

    lane1 = lax.broadcasted_iota(jnp.int32, (1, 128), 1)
    lane512 = lax.broadcasted_iota(jnp.int32, (1, WP), 1)

    def block(fn):
        lax.fori_loop(0, one, lambda _, c: (fn(), c)[1], 0)

    def conv_row(x_ref, valid, taps):
        for ch in range(12):
            rs = pl.ds(16 * ch, 16)
            xp = pltpu.bitcast(x_ref[0, rs, :], U32)
            if valid is None:
                last = jnp.where(lane1 < W - 384, xp[:, 384:], jnp.zeros_like(xp[:, 384:]))
                xp = jnp.concatenate([xp[:, :384], last], axis=1)
            else:
                xp = jnp.where((lane512 < W) & valid, xp, jnp.zeros_like(xp))
            xl = pltpu.roll(xp, 1, 1)
            first = jnp.where(lane1 > 0, xl[:, :128], jnp.zeros_like(xl[:, :128]))
            xl = jnp.concatenate([first, xl[:, 128:]], axis=1)
            xr = pltpu.roll(xp, WP - 1, 1)
            ws = [wtab[k, rs, :] for k in range(9)]
            for s_ in range(4):
                ls = pl.ds(128 * s_, 128)
                xs = [pltpu.bitcast(v[:, 128 * s_:128 * (s_ + 1)], BF16).astype(F32)
                      for v in (xl, xp, xr)]
                for ki, tap in enumerate(taps):
                    if tap is None:
                        continue
                    dst, src = tap
                    t = xs[0] * ws[3 * ki] + xs[1] * ws[3 * ki + 1] + xs[2] * ws[3 * ki + 2]
                    dst[rs, ls] = t if src is None else src[rs, ls] + t

    def layer_norm(x0_row, q):
        for s in range(4):
            ls = pl.ds(128 * s, 128)
            x0 = x0_row[:, ls]
            mean = jnp.sum(x0, axis=0, keepdims=True) * (1.0 / C)
            xc = x0 - mean
            var = jnp.sum(xc * xc, axis=0, keepdims=True) * (1.0 / C)
            hn = xc * lax.rsqrt(var + EPS)
            hs[q][:, ls] = pltpu.pack_elementwise([hn[:96], hn[96:]], packed_dtype=BF16)

    @pl.when(i == 0)
    def _init():
        for k in range(9):
            w = dw_ref[k].astype(F32)
            if k == 4:
                w = w + 1.0
            wtab[k] = w
        src = lax.broadcasted_iota(jnp.int32, (C, C), 0)
        pos = lax.broadcasted_iota(jnp.int32, (C, C), 1)
        p_chan = (src == (pos >> 1) + 96 * (pos & 1)).astype(BF16)
        hp, within = pos // DH, pos % DH
        hd = 2 * (hp % 2) + hp // 2
        p_head = (src == hd * DH + (within >> 1) + 24 * (within & 1)).astype(BF16)
        wt = jnp.dot(wt_ref[...], p_chan, preferred_element_type=F32).astype(BF16)
        r_in, r_hp = src % DH, src // DH
        r_hd = 2 * (r_hp % 2) + r_hp // 2
        p_rows = (pos == r_hd * DH + 2 * (r_in % 24) + r_in // 24).astype(BF16)
        wq = jnp.dot(p_rows, wt[0:C], preferred_element_type=F32)
        wts[0:C, :] = (wq * (DH ** -0.5 * LOG2E)).astype(BF16)
        wts[C:2 * C, :] = wt[C:2 * C]
        wts[2 * C:3 * C, :] = jnp.dot(p_rows, wt[2 * C:3 * C],
                                      preferred_element_type=F32).astype(BF16)
        wos[...] = jnp.dot(wo_ref[...], p_head, preferred_element_type=F32).astype(BF16)
        n0, n1, c0, c1 = x0n.at[0], x0n.at[1], xcs.at[0], xcs.at[1]
        conv_row(x0_ref, None, ((n1, None), (n0, None), None))
        conv_row(x1_ref, None, ((c0, None), (n1, n1), (n0, n0)))
        conv_row(x2_ref, None, ((c1, None), (c0, c0), (n1, n1)))
        layer_norm(n0, 0)

    offs = [((112 * g) // 128, (112 * g) % 128) for g in range(NG)]

    def gather_qv(yh, dst, r, rows, par):
        for g in range(NG):
            a, off = offs[g]
            src = yh[:, 128 * a:128 * (a + 1)]
            if g not in (0, NG - 1):
                src = jnp.where(lane1 >= off, src, yh[:, 128 * (a + 1):128 * (a + 2)])
            idx = jnp.concatenate([pat_ref[_pidx(0, g, r, par)]] * 6, axis=0)
            dst[r, g, rows, :] = jnp.take_along_axis(src, idx, axis=1)

    def qkv_row(r):
        h = pltpu.bitcast(hs[r][...], BF16)
        for s in range(4):
            yk = jnp.dot(wts[C:2 * C, :], h[:, 128 * s:128 * (s + 1)], preferred_element_type=F32)
            kp = pltpu.pack_elementwise([yk[:96], yk[96:]], packed_dtype=BF16)
            blk = jnp.concatenate([kp, jnp.zeros((32, 128), U32)], axis=0)
            kn[r, pl.ds(128 * s, 128), :] = blk.T
        for base, dst in ((0, gq), (2 * C, gv)):
            y2 = jnp.dot(wts[pl.ds(base, C), :], h, preferred_element_type=F32)
            for cls in range(2):
                y = y2[96 * cls:96 * cls + 96]
                yh = jnp.concatenate([
                    pltpu.pack_elementwise([y[48 * hh:48 * hh + 24], y[48 * hh + 24:48 * hh + 48]],
                                           packed_dtype=BF16) for hh in range(2)], axis=0)
                gather_qv(yh, dst, r, pl.ds(48 * cls, 48), cls if base == 0 else 0)

    def part(q):
        if 4 <= q <= 6:
            return x0s.at[q]
        return x0n.at[q - 7] if q in (7, 8) else xcs.at[(q - 2) % WS]

    def final(q):
        if 2 <= q <= 6:
            return x0s.at[q]
        return x0n.at[q % WS]

    for r in range(WS):
        def stage_a(r=r):
            valid = None if r < 4 else (WS * i + 3 + r < H)
            qkv_row(r)
            layer_norm(final(r + 1), (r + 1) % WS)
            if r < 2:
                x0s[r] = x0n[r]
            conv_row(xrows[r], valid, ((part(r + 4), None), (part(r + 3), part(r + 3)),
                                       (final(r + 2), part(r + 2))))
        stage_a()

    masks = (((lane1 >> 3) & 1) == 1, ((lane1 >> 4) & 1) == 1, ((lane1 >> 5) & 1) == 1)
    zero8 = jnp.zeros((8, 128), U32)
    zero24 = jnp.zeros((24, 128), U32)
    zero16 = jnp.zeros((16, 128), U32)
    zero8f = jnp.zeros((8, 128), F32)
    lo = lane1 < 64
    kvalid = (lax.broadcasted_iota(jnp.int32, (56, 128), 0) & 7) < 7

    def regroup(src, dst, g):
        for k in range(12):
            rs = pl.ds(8 * k, 8)
            ins = [src[r, g, rs, :] for r in range(WS)] + [zero8]
            for t, v in enumerate(_barrel(ins, masks, GRP_TILES[g])):
                dst[g, t, rs, :] = v

    def scores(g):
        for t in range(GRP_TILES[g]):
            padslot = (t + 7) % 8
            for pair in range(2):
                qe = dq[g, t, pl.ds(_hpos(2 * pair), 24), :]
                qo = dq[g, t, pl.ds(_hpos(2 * pair + 1), 24), :]
                ra = jnp.concatenate(
                    [jnp.where(lo, qe, zero24), jnp.where(lo, zero24, qo), zero16], axis=0)
                rb = jnp.concatenate(
                    [jnp.where(lo, zero24, qe), jnp.where(lo, qo, zero24), zero16], axis=0)
                for b, rq in ((0, ra), (1, rb)):
                    j = min(16 * g + 2 * t + b, NWIN - 1)
                    pieces = []
                    for s in range(8):
                        r = (s - t) % 8
                        pieces.append(zero8f if r == 7 else pltpu.unpack_elementwise(
                            kn[r, pl.ds(7 * j, 8), :], index=pair, packed_dtype=BF16,
                            unpacked_dtype=F32))
                    kk = jnp.concatenate(pieces, axis=0).astype(BF16)
                    sc = jnp.dot(kk, pltpu.bitcast(rq, BF16), preferred_element_type=F32)
                    scs[g % 2][t, pair, b] = jnp.concatenate(
                        [sc[8 * s:8 * s + 8] for s in range(8) if s != padslot], axis=0)

    def softmax_pv(g):
        for t in range(GRP_TILES[g]):
            padslot = (t + 7) % 8
            for pair in range(2):
                ps, ls_ = [], []
                for b in range(2):
                    sc = jnp.where(kvalid, scs[g % 2][t, pair, b], -jnp.inf)
                    m = jnp.max(sc, axis=0, keepdims=True)
                    p = jnp.exp2(sc - m)
                    ls_.append(jnp.sum(p, axis=0, keepdims=True))
                    blocks, k = [], 0
                    for s in range(8):
                        if s == padslot:
                            blocks.append(zero8f)
                        else:
                            blocks.append(p[8 * k:8 * k + 8])
                            k += 1
                    ps.append(jnp.concatenate(blocks, axis=0))
                for hh in range(2):
                    if hh == 0:
                        pa = jnp.where(lo, ps[0], 0.0)
                        pb = jnp.where(lo, 0.0, ps[1])
                        l = jnp.where(lo, ls_[0], ls_[1])
                    else:
                        pa = jnp.where(lo, 0.0, ps[0])
                        pb = jnp.where(lo, ps[1], 0.0)
                        l = jnp.where(lo, ls_[1], ls_[0])
                    pfull = jnp.concatenate([pa, pb], axis=0).astype(BF16)
                    hrow = pl.ds(_hpos(2 * pair + hh), 24)
                    v = pltpu.bitcast(dv[g, t, hrow, :], BF16)
                    o = jnp.dot(v, pfull, preferred_element_type=F32)
                    rl = pltpu.reciprocal(l, approx=True)
                    rl = rl * (2.0 - l * rl)
                    o = o * rl
                    do[g, t, hrow, :] = pltpu.pack_elementwise(
                        [o[:24], o[24:]], packed_dtype=BF16)

    def inverse(g):
        for k in range(12):
            rs = pl.ds(8 * k, 8)
            ins = [do[g, t, rs, :] if t < GRP_TILES[g] else zero8 for t in range(8)]
            for r, v in enumerate(_barrel(ins, masks, WS)):
                ob[g, r, rs, :] = v
        for r in range(WS):
            for par in range(2):
                rows = pl.ds(48 * par, 48)
                idx = jnp.concatenate([pat_ref[_pidx(1, g, r, par)]] * 6, axis=0)
                res[r, g, rows, :] = jnp.take_along_axis(ob[g, r, rows, :], idx, axis=1)

    def out_proj(rows):
        bounds = (112, 96, 80, 64)
        for r in rows:
            tiles = [jnp.where(lane1 < bounds[s], res[r, s], res[r, s + 1]) for s in range(4)]
            oimg = pltpu.bitcast(jnp.concatenate(tiles, axis=1), BF16)
            y = jnp.dot(wos[...], oimg, preferred_element_type=F32)
            o_ref[r] = (y + x0s[r]).astype(o_ref.dtype)

    for g in range(NG):
        regroup(gq, dq, g)
    for g in range(NG):
        regroup(gv, dv, g)
    scores(0)
    def stage_b(g):
        if g + 1 < NG:
            scores(g + 1)
        softmax_pv(g)

    block(lambda: (stage_b(0), stage_b(1), stage_b(2)))
    stage_b(3)
    stage_b(4)
    for g in range(NG):
        inverse(g)
    out_proj(range(WS))


@jax.jit
def pallas_standalone__window_attn_davit__vision_kernel(x, dw_pe, w_qkv, w_o):
    B, Hh, Ww, Cc = x.shape
    assert (B, Hh, Ww, Cc) == (1, H, W, C)
    xt = jnp.transpose(x, (0, 1, 3, 2)).reshape(H, C, W)
    dwb = jnp.broadcast_to(dw_pe.reshape(9, C, 1), (9, C, 128))
    wt = jnp.transpose(w_qkv)
    wo = jnp.transpose(w_o)
    pat = jnp.asarray(_pattern_table())

    def row_spec(k):
        return pl.BlockSpec((1, C, WP), lambda i: (jnp.minimum(WS * i + 3 + k, H - 1), 0, 0))

    out = pl.pallas_call(
        _kernel,
        grid=(NSTRIP,),
        in_specs=[
            pl.BlockSpec((1, C, WP), lambda i: (0, 0, 0)),
            pl.BlockSpec((1, C, WP), lambda i: (1, 0, 0)),
            pl.BlockSpec((1, C, WP), lambda i: (2, 0, 0)),
            *[row_spec(k) for k in range(WS)],
            pl.BlockSpec((9, C, 128), lambda i: (0, 0, 0)),
            pl.BlockSpec((3 * C, C), lambda i: (0, 0)),
            pl.BlockSpec((C, C), lambda i: (0, 0)),
            pl.BlockSpec(pat.shape, lambda i: (0, 0, 0)),
        ],
        out_specs=pl.BlockSpec((WS, C, WP), lambda i: (i, 0, 0)),
        out_shape=jax.ShapeDtypeStruct((H, C, W), x.dtype),
        scratch_shapes=[
            pltpu.VMEM((9, C, 128), F32),
            pltpu.VMEM((3 * C, C), BF16),
            pltpu.VMEM((C, C), BF16),
            pltpu.VMEM((WS, C, WP), F32),
            pltpu.VMEM((2, C, WP), F32),
            pltpu.VMEM((2, C, WP), F32),
            *[pltpu.VMEM((C // 2, WP), U32)] * 3,
            pltpu.VMEM((WS, NG, 96, 128), U32),
            pltpu.VMEM((WS, NG, 96, 128), U32),
            pltpu.VMEM((WS, WP, 128), U32),
            pltpu.VMEM((NG, 8, 96, 128), U32),
            pltpu.VMEM((NG, 8, 96, 128), U32),
            pltpu.VMEM((NG, 8, 96, 128), U32),
            *[pltpu.VMEM((8, 2, 2, 56, 128), F32)] * 2,
            pltpu.VMEM((WS, NG, 96, 128), U32),
            pltpu.VMEM((NG, WS, 96, 128), U32),
        ],
        compiler_params=pltpu.CompilerParams(
            dimension_semantics=("arbitrary",),
            vmem_limit_bytes=100 * 1024 * 1024,
        ),
    )(*([xt] * (WS + 3)), dwb, wt, wo, pat)
    return jnp.transpose(out.reshape(1, H, C, W), (0, 1, 3, 2))
```
